```python
import os as _os
_os.environ.setdefault("JAX_PLATFORMS", "cpu")
import jax
import jax.numpy as jnp

def _softmax(x, axis=-1):
    return jax.nn.softmax(x, axis=axis)
def _gelu(x):
    return jax.nn.gelu(x, approximate=True)
def _silu(x):
    return jax.nn.silu(x)
def _sigmoid(x):
    return jax.nn.sigmoid(x)
def _layernorm(x, axis=-1, eps=1e-5):
    m = jnp.mean(x, axis=axis, keepdims=True)
    v = jnp.var(x, axis=axis, keepdims=True)
    return (x - m) / jnp.sqrt(v + eps)
def _scatter_add(tgt, idx, src, axis=0):
    return tgt.at[idx].add(src)
def _segment_sum(src, seg, n):
    return jax.ops.segment_sum(src, seg, n)
class _Rng:
    def __init__(self, key):
        self._k = key
    def _next(self):
        self._k, sub = jax.random.split(self._k)
        return sub
    def normal(self, shape):
        return jax.random.normal(self._next(), shape, dtype=jnp.bfloat16)
    def randint(self, lo, hi, shape):
        return jax.random.randint(self._next(), shape, lo, hi, dtype=jnp.int32)
    def uniform(self, shape, lo=0.0, hi=1.0):
        return jax.random.uniform(self._next(), shape, jnp.bfloat16, lo, hi)
    def permutation(self, n):
        return jax.random.permutation(self._next(), n)


kernel_name = 'gated_mix__mha_block__linear_kernel_hedgehog__prompt'

def setup_inputs():
    _rng = _Rng(jax.random.key(int.from_bytes(__import__("os").urandom(4), "little")))
    _w = (lambda a: (lambda t: t.astype(jnp.bfloat16) if jnp.issubdtype(t.dtype, jnp.floating) else t)(jnp.asarray(a)))
    def _A_setup():
        B, S, D, H = 1, 2048, 640, 32
        return {
            "x": _w((lambda *s: _rng.normal(s) * 0.05)(B, S, D)),
            "wqkv": _w((lambda *s: _rng.normal(s) * 0.4)(D, 3 * D)),
            "wo": _w((lambda *s: _rng.normal(s) * 0.05)(D, D)),
        }
    _A_in = _A_setup()

    def _B_setup():
        B, S, D, H = 1, 2048, 640, 32
        Dh = D // H
        return {
            "x": _w((lambda *s: _rng.normal(s) * 0.05)(B, S, D)),
            "wqkv": _w((lambda *s: _rng.normal(s) * 0.8)(D, 3 * D)),
            "w_phi": _w((lambda *s: _rng.normal(s) * 0.8)(H, Dh, Dh) * (Dh ** -0.5)),
            "wo": _w((lambda *s: _rng.normal(s) * 0.05)(D, D)),
        }
    _B_in = _B_setup()

    return {
        "A_x": _A_in["x"],
        "A_wqkv": _A_in["wqkv"],
        "A_wo": _A_in["wo"],
        "B_x": _B_in["x"],
        "B_wqkv": _B_in["wqkv"],
        "B_w_phi": _B_in["w_phi"],
        "B_wo": _B_in["wo"],
        "gate_w": _w((lambda *s: _rng.normal(s) * 0.05)(640) * 16.0),
    }

def reference(A_x, A_wqkv, A_wo, B_x, B_wqkv, B_w_phi, B_wo, gate_w):
    def _A_ref(x, wqkv, wo):
        B, S, D = x.shape
        H = 32
        Dh = D // H
        qkv = (lambda x, *d: x.transpose(*d))((x @ wqkv).reshape(B, S, 3, H, Dh), 2, 0, 3, 1, 4)
        q, k, v = qkv[0], qkv[1], qkv[2]
        scores = jnp.einsum("bhqd,bhkd->bhqk", q, k) * (Dh ** -0.5)
        p = _softmax(scores, axis=-1)
        o = jnp.einsum("bhqk,bhkd->bhqd", p, v)
        return (lambda x, *d: x.transpose(*d))(o, 0, 2, 1, 3).reshape(B, S, D) @ wo

    def _B_ref(x, wqkv, w_phi, wo):
        B, S, D = x.shape
        H = 32; Dh = D // H
        qkv = (lambda x, *d: x.transpose(*d))((x @ wqkv).reshape(B, S, 3, H, Dh), 2, 0, 3, 1, 4)
        q, k, v = qkv[0], qkv[1], qkv[2]
        pq = jnp.einsum("bhsd,hdf->bhsf", q, w_phi)
        pk = jnp.einsum("bhsd,hdf->bhsf", k, w_phi)
        phi_q = jnp.concatenate([_softmax(pq, axis=-1), _softmax(-pq, axis=-1)], axis=-1)
        phi_k = jnp.concatenate([_softmax(pk, axis=-1), _softmax(-pk, axis=-1)], axis=-1)
        kv = jnp.einsum("bhsf,bhsd->bhfd", phi_k, v)
        z  = jnp.einsum("bhsf->bhf", phi_k)
        num = jnp.einsum("bhqf,bhfd->bhqd", phi_q, kv)
        den = jnp.einsum("bhqf,bhf->bhq", phi_q, z)[..., None] + 1e-6
        o = num / den
        return (lambda x, *d: x.transpose(*d))(o, 0, 2, 1, 3).reshape(B, S, D) @ wo

    x = A_x
    g = _sigmoid((x * gate_w).sum(-1, keepdims=True))
    a = _A_ref(x, A_wqkv, A_wo)
    b = _B_ref(x, B_wqkv, B_w_phi, B_wo)
    return g * a + (1 - g) * b
```

```python
import functools
import jax
import jax.numpy as jnp
from jax import lax
from jax.experimental import pallas as pl
from jax.experimental.pallas import tpu as pltpu

S, D, H, DH = 2048, 640, 32, 20
LOG2E = 1.4426950408889634
QSCALE = (DH ** -0.5) * LOG2E
F32, BF16 = jnp.float32, jnp.bfloat16
NT = (((1,), (1,)), ((), ()))
TN = (((0,), (0,)), ((), ()))
R_QA, R_VA, R_PQ, R_PK, R_VB, R_G, R_END = 0, 640, 1280, 1920, 2560, 3200, 3232
HALF = R_END // 2
CH = 512
NCH = S // CH
KT, NKT = 108, 19
SP = 2080
VP = 2176
U32 = jnp.uint32
HS = S // 2
SCORE_LIMIT = 56.0
V_LO, V_HI = 2.0 ** -36, 2.0 ** 50


def _iota(shape, dim):
    return lax.broadcasted_iota(jnp.int32, shape, dim)


def _dot(a, b):
    return jnp.dot(a, b, preferred_element_type=F32)


def _dot_nt(a, b):
    return lax.dot_general(a, b, NT, preferred_element_type=F32)


def _feat_tile(x, seed=None):
    L = x.shape[1]
    x3 = x.reshape(5, 8, L)

    def allred(v, op):
        v = op(v, pltpu.roll(v, 2, 0))
        return op(v, pltpu.roll(v, 4, 0))
    mx = jnp.max(x3, axis=0)
    mn = jnp.min(x3, axis=0)
    if seed is not None:
        mx = mx + seed
        mn = mn + seed
    mx = allred(mx, jnp.maximum)
    mn = allred(mn, jnp.minimum)
    ep = jnp.exp2(x3 - mx[None])
    en = jnp.exp2(mn[None] - x3)
    rp = 1.0 / allred(jnp.sum(ep, axis=0), jnp.add)
    rn = 1.0 / allred(jnp.sum(en, axis=0), jnp.add)
    return jnp.concatenate([(ep * rp[None]).reshape(40, L), (en * rn[None]).reshape(40, L)],
                           axis=0).astype(BF16)


def _kernel(x_hbm, wa_hbm, woa_hbm, wb_hbm, phi_ref, wob_hbm, gate_ref, out_hbm,
            x_ref, wa_ref, wb_ref, woa_ref, wob_ref, ob_ref, sems, osems,
            wt_ref, yt_ref, ks_ref, ota_ref, otb_ref,
            phi2_ref, g_ref, am_ref, km_ref, m_ref, w0_ref, l0_ref, ao_ref, al_ref):
    c_wk = pltpu.make_async_copy(wa_hbm.at[:, pl.ds(D, D)], wa_ref.at[:, pl.ds(D, D)], sems.at[0])
    c_x0 = pltpu.make_async_copy(x_hbm.at[pl.ds(0, CH), :], x_ref.at[pl.ds(0, CH), :], sems.at[1])
    c_x1 = pltpu.make_async_copy(x_hbm.at[pl.ds(CH, S - CH), :], x_ref.at[pl.ds(CH, S - CH), :], sems.at[2])
    c_wq = pltpu.make_async_copy(wa_hbm.at[:, pl.ds(0, D)], wa_ref.at[:, pl.ds(0, D)], sems.at[3])
    c_wv = pltpu.make_async_copy(wa_hbm.at[:, pl.ds(2 * D, D)], wa_ref.at[:, pl.ds(2 * D, D)], sems.at[4])
    c_wb = pltpu.make_async_copy(wb_hbm, wb_ref, sems.at[5])
    c_woa = pltpu.make_async_copy(woa_hbm, woa_ref, sems.at[6])
    c_wob = pltpu.make_async_copy(wob_hbm, wob_ref, sems.at[7])
    for c in (c_wk, c_x0, c_x1, c_wq, c_wv, c_wb, c_woa, c_wob):
        c.start()

    for d in range(DH):
        pt = phi_ref[d].astype(F32).T
        phi2_ref[pl.ds(d, H, stride=DH), :] = jnp.concatenate(
            [pt, jnp.zeros((H, 128 - DH), F32)], axis=1)

    def proj_k(r0, n):
        k = _dot(x_ref[r0:r0 + n, :], wa_ref[:, D:2 * D])
        ks_ref[r0:r0 + n, :] = k.astype(BF16)
        return jnp.max(jnp.abs(k).reshape(n // 8, 8, D), axis=0)
    ks_ref[S:SP, :] = jnp.zeros((SP - S, D), BF16)
    c_wk.wait()
    c_x0.wait()
    km0 = proj_k(0, CH)
    c_x1.wait()
    km1 = proj_k(CH, S - CH)
    km_ref[...] = jnp.maximum(km0, km1)

    c_wq.wait()
    c_wv.wait()
    c_wb.wait()
    wt_ref[R_QA:R_QA + D, :] = wa_ref[:, 0:D].T
    wt_ref[R_VA:R_VA + D, :] = wa_ref[:, 2 * D:3 * D].T
    wt_ref[R_VB:R_VB + D, :] = wb_ref[:, 2 * D:3 * D].T
    grow = jnp.broadcast_to(gate_ref[...].astype(F32).reshape(1, D), (32, D))
    wt_ref[R_G:R_END, :] = jnp.where(_iota((32, D), 0) == 0, grow, 0.0).astype(BF16)

    ri = _iota((128, 128), 0)
    ci = _iota((128, 128), 1)
    sel = ((ri % 40) // 2 == ci).astype(BF16)
    keep = (2 * (ri // 40) + ri % 2 == ci // DH) & (ri < 120)
    for g in range(6):
        n = 120 if g < 5 else 40
        c0 = min(120 * g, D - 128)
        pw = phi2_ref[c0:c0 + 128, :].astype(BF16)
        rep = _dot_nt(sel, pw)
        if g < 5:
            kp = keep
        else:
            kp = (30 + 2 * (ri // 40) + ri % 2 == (c0 + ci) // DH) & (ri < 40)
        lg = jnp.where(kp, rep, 0.0).astype(BF16)
        for col0, r0 in ((0, R_PQ), (D, R_PK)):
            fold = _dot_nt(lg, wb_ref[:, col0 + c0:col0 + c0 + 128]) * LOG2E
            yt_ref[r0 - R_PQ + 120 * g:r0 - R_PQ + 120 * g + n, 0:D] = fold[0:n]
    wt_ref[R_PQ:R_VB, :] = yt_ref[0:2 * D, 0:D].astype(BF16)

    def proj_t(i, c):
        j = i // 2
        r = pl.multiple_of((i % 2) * HALF, 16)
        off = pl.multiple_of(j * CH, CH)
        y = _dot_nt(wt_ref[pl.ds(r, HALF), :], x_ref[pl.ds(off, CH), :])
        yt_ref[pl.ds(r, HALF), pl.ds(off, CH)] = y
        ay = jnp.abs(y)
        am = functools.reduce(jnp.maximum, [ay[:, 128 * t:128 * (t + 1)] for t in range(CH // 128)])
        am_ref[pl.ds(r, HALF), :] = jnp.where(j == 0, am, jnp.maximum(am, am_ref[pl.ds(r, HALF), :]))
        return c
    am_ref[...] = jnp.zeros(am_ref.shape, F32)
    lax.fori_loop(0, 2 * NCH, proj_t, 0)

    kmax = jnp.max(km_ref[...], axis=0, keepdims=True)
    seg = _iota((H, D), 1) // DH == _iota((H, D), 0)
    amat = jnp.where(seg, jnp.broadcast_to(kmax, (H, D)), 0.0).astype(BF16)
    bound = jnp.max(_dot(amat, (am_ref[R_QA:R_QA + D, :] * QSCALE).astype(BF16)))
    vmax = jnp.max(am_ref[R_VA:R_VA + D, :])
    safe = (bound <= SCORE_LIMIT) & (vmax >= V_LO) & (vmax <= V_HI)

    g_ref[...] = jnp.broadcast_to(jax.nn.sigmoid(yt_ref[R_G:R_G + 1, :]), (8, S))

    mr = _iota((48, 80), 0)
    mkeep = jnp.where(mr < 40, mr // DH, mr - 40) == _iota((48, 80), 1) % 2

    def hh_lv(o40, c0, n):
        ones8 = jnp.where(_iota((8, n), 0) < 2, 1.0, 0.0)
        return jnp.concatenate([yt_ref[pl.ds(R_VB + o40, 40), pl.ds(c0, n)], ones8], axis=0).astype(BF16)

    def hh_out(nd, o40, c0, n):
        omg = 1.0 - g_ref[0:1, pl.ds(c0, n)]
        s0 = omg / (nd[40:41, :] + 1e-6)
        s1 = omg / (nd[41:42, :] + 1e-6)
        otb_ref[pl.ds(o40, 40), pl.ds(c0, n)] = nd[0:40, :] * jnp.where(_iota((40, n), 0) < DH, s0, s1)

    def head_rows(r0, hd):
        lo = hd * DH
        w32 = yt_ref[pl.ds(pl.multiple_of(r0 + (lo // 8) * 8, 8), 32), :]
        return jnp.where(hd % 2 == 1, w32[4:28], w32[0:24])

    def head_geom(h):
        lo = h * DH
        a = lo // 128
        return (pl.multiple_of(a * 128, 128), pl.multiple_of(jnp.minimum(a + 1, 4) * 128, 128),
                lo - a * 128)

    @pl.when(safe)
    def _():
        sub8 = _iota((8, S), 0)
        lane = _iota((1, 128), 1)

        def q_rows(hd):
            qf = head_rows(R_QA, hd) * QSCALE
            return pltpu.roll(qf[0:8], 4, 0), qf[4:20]

        def v_rows(hd):
            return jnp.concatenate([head_rows(R_VA, hd)[0:DH], jnp.zeros((DH, VP - S), F32)], axis=1)

        def make_lhs(hk, tk, vf, tv, seed=None):
            ca, cb, off = head_geom(hk)
            r0 = (KT * tk) // 16 * 16
            o = KT * tk - r0
            ka = ks_ref[r0:r0 + 128, pl.ds(ca, 128)].astype(F32)[o:o + KT]
            kb = ks_ref[r0:r0 + 128, pl.ds(cb, 128)].astype(F32)[o:o + KT]
            kp = jnp.where(lane >= off, ka, kb)
            if seed is not None:
                kp = kp + seed
            kp = pltpu.roll(kp, (KT + 128 - off) % 128, 1)
            kp = jnp.where(lane >= KT, kp, 0.0)
            if vf is not None:
                vp = jnp.where(lane < KT, vf[:, KT * tv:KT * tv + 128], 0.0)
            else:
                vp = jnp.zeros((DH, 128), F32)
            return jnp.concatenate([kp, vp], axis=0).astype(BF16)

        def make_w(e, qt, qb):
            return jnp.concatenate([e[0:104], jnp.where(sub8 < 4, e[104:112], qt), qb], axis=0).astype(BF16)

        def fin(ao, al, slot):
            inv = g_ref[0:1, :] / jnp.sum(al, axis=0, keepdims=True)
            ota_ref[slot] = ao * inv

        qt0, qb0 = q_rows(0)
        w0_ref[...] = make_w(jnp.zeros((112, S), F32), qt0, qb0)
        l0_ref[...] = make_lhs(0, 0, None, 0)
        ao_ref[...] = jnp.zeros(ao_ref.shape, F32)
        al_ref[...] = jnp.ones(al_ref.shape, F32)
        m_ref[...] = jnp.zeros(m_ref.shape, F32)

        def head(h, c):
            hn = jnp.minimum(h + 1, H - 1)
            qt, qb = q_rows(h)
            vf = v_rows(h)
            pk = h // 2
            pq = jnp.maximum(pk - 1, 0)
            c0 = pl.multiple_of((h % 2) * HS, HS)
            ok = pl.multiple_of(pk * 40, 8)
            oq = pl.multiple_of(pq * 40, 8)
            fq, fk = [], []
            w = w0_ref[...]
            lhs = l0_ref[...]
            ao, al = ao_ref[...], al_ref[...]
            prev = None
            for t in range(NKT):
                out = _dot(lhs, w)
                seed = None if prev is None else prev[0:8, 0:128] * 0.0
                useed = None if seed is None else seed[0:1]
                if t + 1 < NKT:
                    lhs = make_lhs(h, t + 1, vf, t, useed)
                else:
                    lhs = make_lhs(hn, 0, vf, t, useed)
                ao = ao + out[104:128]
                if t == 0:
                    fin(ao, al, h)
                    ao = jnp.zeros((24, S), F32)
                    al = None
                e = jnp.exp2(out[0:112])
                last = e[104:112]
                last = jnp.where(sub8 < (4 if t + 1 < NKT else 0), last, 0.0)
                tot = functools.reduce(jnp.add, [e[8 * i:8 * i + 8] for i in range(13)] + [last])
                al = tot if al is None else al + tot
                if t + 1 < NKT:
                    w = make_w(e, qt, qb)
                else:
                    w = make_w(e, *q_rows(hn))
                if seed is not None and t <= 8:
                    u = len(fq)
                    fq.append(_feat_tile(yt_ref[pl.ds(R_PQ + oq, 40), pl.ds(c0 + 128 * u, 128)], seed))
                elif 9 <= t <= 16:
                    u = len(fk)
                    fk.append(_feat_tile(yt_ref[pl.ds(R_PK + ok, 40), pl.ds(c0 + 128 * u, 128)], seed))
                prev = out
            hh_out(_dot(m_ref[pq].astype(BF16), jnp.concatenate(fq, axis=1)), oq, c0, HS)
            kv = _dot_nt(hh_lv(ok, c0, HS), jnp.concatenate(fk, axis=1))
            kv = jnp.where(mkeep, kv, 0.0)
            m_ref[pk] = jnp.where(h % 2 == 0, kv, kv + m_ref[pk])
            w0_ref[...] = w
            l0_ref[...] = lhs
            ao_ref[...] = ao
            al_ref[...] = al
            return c
        lax.fori_loop(0, H, head, 0)
        out = _dot(l0_ref[...], w0_ref[...])
        fin(ao_ref[...] + out[104:128], al_ref[...], H)
        o40 = (H // 2 - 1) * 40
        hh_out(_dot(m_ref[H // 2 - 1].astype(BF16), _feat_tile(yt_ref[R_PQ + o40:R_PQ + o40 + 40, :])), o40, 0, S)

    @pl.when(jnp.logical_not(safe))
    def _():
        def pair(p, c):
            o40 = pl.multiple_of(p * 40, 8)
            kv = _dot_nt(hh_lv(o40, 0, S), _feat_tile(yt_ref[pl.ds(R_PK + o40, 40), :]))
            m = jnp.where(mkeep, kv, 0.0).astype(BF16)
            hh_out(_dot(m, _feat_tile(yt_ref[pl.ds(R_PQ + o40, 40), :])), o40, 0, S)
            return c
        lax.fori_loop(0, H // 2, pair, 0)

        def slow(i, c):
            h = i // (S // 256)
            c0 = pl.multiple_of((i % (S // 256)) * 256, 256)
            ca, cb, off = head_geom(h)
            s = None
            for cw, first in ((ca, True), (cb, False)):
                rows = _iota((128, 256), 0) + (off * 0 if first else 128)
                msk = (rows >= off) & (rows < off + DH)
                if not first:
                    msk = msk & (cb != ca)
                qm = jnp.where(msk, yt_ref[pl.ds(cw, 128), pl.ds(c0, 256)] * QSCALE, 0.0).astype(BF16)
                part = _dot(ks_ref[0:S, pl.ds(cw, 128)], qm)
                s = part if s is None else s + part
            p = jnp.exp2(s - jnp.max(s, axis=0, keepdims=True)).astype(BF16)
            vf = head_rows(R_VA, h)[0:DH]
            c256 = jnp.concatenate([vf, jnp.where(_iota((12, S), 0) == 0, 1.0, 0.0)], axis=0).astype(BF16)
            o = _dot(c256, p)
            o = jnp.concatenate([o[28:32], o[0:DH]], axis=0) * (g_ref[0:1, pl.ds(c0, 256)] / o[DH:DH + 1])
            ota_ref[h + 1, :, pl.ds(c0, 256)] = o
            return c
        lax.fori_loop(0, H * (S // 256), slow, 0)

    c_woa.wait()
    c_wob.wait()

    def ocopy(j):
        return pltpu.make_async_copy(ob_ref.at[j], out_hbm.at[pl.ds(j * CH, CH), :], osems.at[j])
    for j in range(NCH):
        off = j * CH
        oa = jnp.concatenate([ota_ref[h + 1, 4:4 + DH, off:off + CH] for h in range(H)], axis=0).astype(BF16)
        r = lax.dot_general(oa, woa_ref[...], TN, preferred_element_type=F32)
        r = r + lax.dot_general(otb_ref[:, off:off + CH].astype(BF16), wob_ref[...], TN,
                                preferred_element_type=F32)
        ob_ref[j] = r.astype(BF16)
        ocopy(j).start()
    for j in range(NCH):
        ocopy(j).wait()


@jax.jit
def pallas_gated_mix__mha_block__linear_kernel_hedgehog__prompt_kernel(
    A_x, A_wqkv, A_wo, B_x, B_wqkv, B_w_phi, B_wo, gate_w
):
    x = A_x.reshape(S, D)
    hbm = pl.BlockSpec(memory_space=pl.ANY)
    vmem = pl.BlockSpec(memory_space=pltpu.VMEM)
    out = pl.pallas_call(
        _kernel,
        out_shape=jax.ShapeDtypeStruct((S, D), BF16),
        in_specs=[hbm, hbm, hbm, hbm, vmem, hbm, vmem],
        out_specs=hbm,
        scratch_shapes=[
            pltpu.VMEM((S, D), BF16),
            pltpu.VMEM((D, 3 * D), BF16),
            pltpu.VMEM((D, 3 * D), BF16),
            pltpu.VMEM((D, D), BF16),
            pltpu.VMEM((D, D), BF16),
            pltpu.VMEM((NCH, CH, D), BF16),
            pltpu.SemaphoreType.DMA((8,)),
            pltpu.SemaphoreType.DMA((NCH,)),
            pltpu.VMEM((R_END, D), BF16),
            pltpu.VMEM((R_END, S), F32),
            pltpu.VMEM((SP, D), BF16),
            pltpu.VMEM((H + 1, 24, S), F32),
            pltpu.VMEM((D, S), F32),
            pltpu.VMEM((D, 128), F32),
            pltpu.VMEM((8, S), F32),
            pltpu.VMEM((R_END, 128), F32),
            pltpu.VMEM((8, D), F32),
            pltpu.VMEM((H // 2, 48, 80), F32),
            pltpu.VMEM((128, S), BF16),
            pltpu.VMEM((128, 128), BF16),
            pltpu.VMEM((24, S), F32),
            pltpu.VMEM((8, S), F32),
        ],
        compiler_params=pltpu.CompilerParams(vmem_limit_bytes=120 * 1024 * 1024),
    )(x, A_wqkv, A_wo, B_wqkv, jnp.transpose(B_w_phi, (1, 2, 0)), B_wo, gate_w)
    return out.reshape(1, S, D)
```

```python
import functools
import jax
import jax.numpy as jnp
from jax import lax
from jax.experimental import pallas as pl
from jax.experimental.pallas import tpu as pltpu

S, D, H, DH = 2048, 640, 32, 20
LOG2E = 1.4426950408889634
QSCALE = (DH ** -0.5) * LOG2E
F32, BF16 = jnp.float32, jnp.bfloat16
NT = (((1,), (1,)), ((), ()))
TN = (((0,), (0,)), ((), ()))
R_QA, R_VA, R_PQ, R_PK, R_VB, R_G, R_END = 0, 640, 1280, 1920, 2560, 3200, 3216
CH = 512
NCH = S // CH
KT, NKT = 108, 19
SP = 2080
VP = 2176
OCH = ((0, 512), (512, 1024), (1024, 1536), (1536, 1920), (1920, 2048))
HS = S // 2
SCORE_LIMIT = 56.0
V_LO, V_HI = 2.0 ** -36, 2.0 ** 50


def _iota(shape, dim):
    return lax.broadcasted_iota(jnp.int32, shape, dim)


def _dot(a, b):
    return jnp.dot(a, b, preferred_element_type=F32)


def _dot_nt(a, b):
    return lax.dot_general(a, b, NT, preferred_element_type=F32)


def _feat_tile(x, seed=None):
    L = x.shape[1]
    x3 = x.reshape(5, 8, L)

    def allred(v, op):
        v = op(v, pltpu.roll(v, 2, 0))
        return op(v, pltpu.roll(v, 4, 0))
    mx = jnp.max(x3, axis=0)
    mn = jnp.min(x3, axis=0)
    if seed is not None:
        mx = mx + seed
        mn = mn + seed
    mx = allred(mx, jnp.maximum)
    mn = allred(mn, jnp.minimum)
    ep = jnp.exp2(x3 - mx[None])
    en = jnp.exp2(mn[None] - x3)
    rp = 1.0 / allred(jnp.sum(ep, axis=0), jnp.add)
    rn = 1.0 / allred(jnp.sum(en, axis=0), jnp.add)
    return jnp.concatenate([(ep * rp[None]).reshape(40, L), (en * rn[None]).reshape(40, L)],
                           axis=0).astype(BF16)


def _kernel(x_hbm, wa_hbm, woa_hbm, wb_hbm, phi_hbm, wob_hbm, gate_hbm, out_hbm,
            x_ref, wq_ref, wk_ref, wv_ref, wb_ref, woa_ref, wob_ref, phi_ref, gate_ref, ob_ref, sems, osems,
            wt_ref, yt_ref, ks_ref, ota_ref, otb_ref,
            phi2_ref, g_ref, am_ref, km_ref, m_ref, w0_ref, l0_ref, ao_ref, al_ref):
    X0, X1 = CH, 1792

    def xcopy(r0, r1, k):
        return pltpu.make_async_copy(x_hbm.at[pl.ds(r0, r1 - r0), :], x_ref.at[pl.ds(r0, r1 - r0), :], sems.at[k])
    c_wk = pltpu.make_async_copy(wa_hbm.at[:, pl.ds(D, D)], wk_ref, sems.at[0])
    c_x0 = xcopy(0, X0, 1)
    c_x1 = xcopy(X0, X1, 2)
    c_phi = pltpu.make_async_copy(phi_hbm, phi_ref, sems.at[3])
    c_gate = pltpu.make_async_copy(gate_hbm, gate_ref, sems.at[4])
    c_wq = pltpu.make_async_copy(wa_hbm.at[:, pl.ds(0, D)], wq_ref, sems.at[5])
    c_wv = pltpu.make_async_copy(wa_hbm.at[:, pl.ds(2 * D, D)], wv_ref, sems.at[6])
    c_wb = pltpu.make_async_copy(wb_hbm, wb_ref, sems.at[7])
    c_x2 = xcopy(X1, S, 8)
    c_woa = pltpu.make_async_copy(woa_hbm, woa_ref, sems.at[9])
    c_wob = pltpu.make_async_copy(wob_hbm, wob_ref, sems.at[10])
    for c in (c_wk, c_x0, c_x1, c_phi, c_gate, c_wq, c_wv, c_wb, c_x2, c_woa, c_wob):
        c.start()

    def proj_k(r0, n):
        km = None
        for q in range(4):
            a, b = r0 + q * n // 4, r0 + (q + 1) * n // 4
            k = _dot(x_ref[a:b, :], wk_ref[...])
            ks_ref[a:b, :] = k.astype(BF16)
            m = jnp.max(jnp.abs(k).reshape((b - a) // 8, 8, D), axis=0)
            km = m if km is None else jnp.maximum(km, m)
        return km
    ks_ref[S:SP, :] = jnp.zeros((SP - S, D), BF16)
    c_wk.wait()
    c_x0.wait()
    km = proj_k(0, X0)
    c_x1.wait()
    km = jnp.maximum(km, proj_k(X0, X1 - X0))
    for c in (c_phi, c_gate, c_wq, c_wv, c_wb, c_x2):
        c.wait()
    km_ref[...] = jnp.maximum(km, proj_k(X1, S - X1))

    for d in range(DH):
        pt = phi_ref[d].astype(F32).T
        phi2_ref[pl.ds(d, H, stride=DH), :] = jnp.concatenate(
            [pt, jnp.zeros((H, 128 - DH), F32)], axis=1)

    wt_ref[R_QA:R_QA + D, :] = wq_ref[...].T
    wt_ref[R_VA:R_VA + D, :] = wv_ref[...].T
    wt_ref[R_VB:R_VB + D, :] = wb_ref[:, 2 * D:3 * D].T
    grow = jnp.broadcast_to(gate_ref[...].astype(F32).reshape(1, D), (16, D))
    wt_ref[R_G:R_END, :] = jnp.where(_iota((16, D), 0) == 0, grow, 0.0).astype(BF16)

    ri = _iota((128, 128), 0)
    ci = _iota((128, 128), 1)
    sel = ((ri % 40) // 2 == ci).astype(BF16)
    keep = (2 * (ri // 40) + ri % 2 == ci // DH) & (ri < 120)
    for g in range(6):
        n = 120 if g < 5 else 40
        c0 = min(120 * g, D - 128)
        pw = phi2_ref[c0:c0 + 128, :].astype(BF16)
        rep = _dot_nt(sel, pw)
        if g < 5:
            kp = keep
        else:
            kp = (30 + 2 * (ri // 40) + ri % 2 == (c0 + ci) // DH) & (ri < 40)
        lg = jnp.where(kp, rep, 0.0).astype(BF16)
        for col0, r0 in ((0, R_PQ), (D, R_PK)):
            fold = _dot_nt(lg, wb_ref[:, col0 + c0:col0 + c0 + 128]) * LOG2E
            yt_ref[r0 - R_PQ + 120 * g:r0 - R_PQ + 120 * g + n, 0:D] = fold[0:n]
    wt_ref[R_PQ:R_VB, :] = yt_ref[0:2 * D, 0:D].astype(BF16)

    PC = 256

    def proj_t(j, c):
        off = pl.multiple_of(j * PC, PC)
        y = _dot_nt(wt_ref[...], x_ref[pl.ds(off, PC), :])
        yt_ref[:, pl.ds(off, PC)] = y
        ay = jnp.abs(y[0:2 * D])
        am = jnp.maximum(ay[:, 0:128], ay[:, 128:256])
        am_ref[...] = jnp.maximum(am, am_ref[...])
        return c
    am_ref[...] = jnp.zeros(am_ref.shape, F32)
    lax.fori_loop(0, S // PC, proj_t, 0)

    kmax = jnp.max(km_ref[...], axis=0, keepdims=True)
    seg = _iota((H, D), 1) // DH == _iota((H, D), 0)
    amat = jnp.where(seg, jnp.broadcast_to(kmax, (H, D)), 0.0).astype(BF16)
    bound = jnp.max(_dot(amat, (am_ref[R_QA:R_QA + D, :] * QSCALE).astype(BF16)))
    vmax = jnp.max(am_ref[R_VA:R_VA + D, :])
    safe = (bound <= SCORE_LIMIT) & (vmax >= V_LO) & (vmax <= V_HI)

    g_ref[...] = jnp.broadcast_to(jax.nn.sigmoid(yt_ref[R_G:R_G + 1, :]), (8, S))

    mr = _iota((48, 80), 0)
    mkeep = jnp.where(mr < 40, mr // DH, mr - 40) == _iota((48, 80), 1) % 2

    def hh_lv(o40, c0, n):
        ones8 = jnp.where(_iota((8, n), 0) < 2, 1.0, 0.0)
        return jnp.concatenate([yt_ref[pl.ds(R_VB + o40, 40), pl.ds(c0, n)], ones8], axis=0).astype(BF16)

    def hh_out(nd, o40, c0, n):
        omg = 1.0 - g_ref[0:1, pl.ds(c0, n)]
        s0 = omg / (nd[40:41, :] + 1e-6)
        s1 = omg / (nd[41:42, :] + 1e-6)
        otb_ref[pl.ds(o40, 40), pl.ds(c0, n)] = nd[0:40, :] * jnp.where(_iota((40, n), 0) < DH, s0, s1)

    def head_rows(r0, hd):
        lo = hd * DH
        w32 = yt_ref[pl.ds(pl.multiple_of(r0 + (lo // 8) * 8, 8), 32), :]
        return jnp.where(hd % 2 == 1, w32[4:28], w32[0:24])

    def head_geom(h):
        lo = h * DH
        a = lo // 128
        return (pl.multiple_of(a * 128, 128), pl.multiple_of(jnp.minimum(a + 1, 4) * 128, 128),
                lo - a * 128)

    @pl.when(safe)
    def _():
        sub8 = _iota((8, S), 0)
        lane = _iota((1, 128), 1)

        def q_rows(hd):
            qf = head_rows(R_QA, hd) * QSCALE
            return pltpu.roll(qf[0:8], 4, 0), qf[4:20]

        def v_rows(hd):
            return jnp.concatenate([head_rows(R_VA, hd)[0:DH], jnp.zeros((DH, VP - S), F32)], axis=1)

        def make_lhs(hk, tk, vf, tv, seed=None):
            ca, cb, off = head_geom(hk)
            r0 = (KT * tk) // 16 * 16
            o = KT * tk - r0
            ka = ks_ref[r0:r0 + 128, pl.ds(ca, 128)].astype(F32)[o:o + KT]
            kb = ks_ref[r0:r0 + 128, pl.ds(cb, 128)].astype(F32)[o:o + KT]
            kp = jnp.where(lane >= off, ka, kb)
            if seed is not None:
                kp = kp + seed
            kp = pltpu.roll(kp, (KT + 128 - off) % 128, 1)
            kp = jnp.where(lane >= KT, kp, 0.0)
            if vf is not None:
                vp = jnp.where(lane < KT, vf[:, KT * tv:KT * tv + 128], 0.0)
            else:
                vp = jnp.zeros((DH, 128), F32)
            return jnp.concatenate([kp, vp], axis=0).astype(BF16)

        def make_w(e, qt, qb):
            return jnp.concatenate([e[0:104], jnp.where(sub8 < 4, e[104:112], qt), qb], axis=0).astype(BF16)

        def fin(ao, al, slot):
            inv = g_ref[0:1, :] / jnp.sum(al, axis=0, keepdims=True)
            ota_ref[slot] = ao * inv

        qt0, qb0 = q_rows(0)
        w0_ref[...] = make_w(jnp.zeros((112, S), F32), qt0, qb0)
        l0_ref[...] = make_lhs(0, 0, None, 0)
        ao_ref[...] = jnp.zeros(ao_ref.shape, F32)
        al_ref[...] = jnp.ones(al_ref.shape, F32)
        m_ref[...] = jnp.zeros(m_ref.shape, F32)

        def head(h, c):
            hn = jnp.minimum(h + 1, H - 1)
            qt, qb = q_rows(h)
            vf = v_rows(h)
            pk = h // 2
            pq = jnp.maximum(pk - 1, 0)
            c0 = pl.multiple_of((h % 2) * HS, HS)
            ok = pl.multiple_of(pk * 40, 8)
            oq = pl.multiple_of(pq * 40, 8)
            fq, fk = [], []
            w = w0_ref[...]
            lhs = l0_ref[...]
            ao, al = ao_ref[...], al_ref[...]
            prev = None
            for t in range(NKT):
                out = _dot(lhs, w)
                seed = None if prev is None else prev[0:8, 0:128] * 0.0
                useed = None if seed is None else seed[0:1]
                if t + 1 < NKT:
                    lhs = make_lhs(h, t + 1, vf, t, useed)
                else:
                    lhs = make_lhs(hn, 0, vf, t, useed)
                ao = ao + out[104:128]
                if t == 0:
                    fin(ao, al, h)
                    ao = jnp.zeros((24, S), F32)
                    al = None
                e = jnp.exp2(out[0:112])
                last = e[104:112]
                last = jnp.where(sub8 < (4 if t + 1 < NKT else 0), last, 0.0)
                tot = functools.reduce(jnp.add, [e[8 * i:8 * i + 8] for i in range(13)] + [last])
                al = tot if al is None else al + tot
                if t + 1 < NKT:
                    w = make_w(e, qt, qb)
                else:
                    w = make_w(e, *q_rows(hn))
                if seed is not None and t <= 8:
                    u = len(fq)
                    fq.append(_feat_tile(yt_ref[pl.ds(R_PQ + oq, 40), pl.ds(c0 + 128 * u, 128)], seed))
                elif 9 <= t <= 16:
                    u = len(fk)
                    fk.append(_feat_tile(yt_ref[pl.ds(R_PK + ok, 40), pl.ds(c0 + 128 * u, 128)], seed))
                prev = out
            hh_out(_dot(m_ref[pq].astype(BF16), jnp.concatenate(fq, axis=1)), oq, c0, HS)
            kv = _dot_nt(hh_lv(ok, c0, HS), jnp.concatenate(fk, axis=1))
            kv = jnp.where(mkeep, kv, 0.0)
            m_ref[pk] = jnp.where(h % 2 == 0, kv, kv + m_ref[pk])
            w0_ref[...] = w
            l0_ref[...] = lhs
            ao_ref[...] = ao
            al_ref[...] = al
            return c
        lax.fori_loop(0, H, head, 0)
        out = _dot(l0_ref[...], w0_ref[...])
        fin(ao_ref[...] + out[104:128], al_ref[...], H)

    @pl.when(jnp.logical_not(safe))
    def _():
        def pair(p, c):
            o40 = pl.multiple_of(p * 40, 8)
            kv = _dot_nt(hh_lv(o40, 0, S), _feat_tile(yt_ref[pl.ds(R_PK + o40, 40), :]))
            m = jnp.where(mkeep, kv, 0.0)
            m_ref[p] = m
            hh_out(_dot(m.astype(BF16), _feat_tile(yt_ref[pl.ds(R_PQ + o40, 40), :])), o40, 0, S)
            return c
        lax.fori_loop(0, H // 2, pair, 0)

        def slow(i, c):
            h = i // (S // 256)
            c0 = pl.multiple_of((i % (S // 256)) * 256, 256)
            ca, cb, off = head_geom(h)
            s = None
            for cw, first in ((ca, True), (cb, False)):
                rows = _iota((128, 256), 0) + (off * 0 if first else 128)
                msk = (rows >= off) & (rows < off + DH)
                if not first:
                    msk = msk & (cb != ca)
                qm = jnp.where(msk, yt_ref[pl.ds(cw, 128), pl.ds(c0, 256)] * QSCALE, 0.0).astype(BF16)
                part = _dot(ks_ref[0:S, pl.ds(cw, 128)], qm)
                s = part if s is None else s + part
            p = jnp.exp2(s - jnp.max(s, axis=0, keepdims=True)).astype(BF16)
            vf = head_rows(R_VA, h)[0:DH]
            c256 = jnp.concatenate([vf, jnp.where(_iota((12, S), 0) == 0, 1.0, 0.0)], axis=0).astype(BF16)
            o = _dot(c256, p)
            o = jnp.concatenate([o[28:32], o[0:DH]], axis=0) * (g_ref[0:1, pl.ds(c0, 256)] / o[DH:DH + 1])
            ota_ref[h + 1, :, pl.ds(c0, 256)] = o
            return c
        lax.fori_loop(0, H * (S // 256), slow, 0)

    c_woa.wait()
    c_wob.wait()
    def ocopy(j):
        r0, r1 = OCH[j]
        return pltpu.make_async_copy(ob_ref.at[pl.ds(r0, r1 - r0), :], out_hbm.at[pl.ds(r0, r1 - r0), :], osems.at[j])
    for j, (r0, r1) in enumerate(OCH):
        oa = jnp.concatenate([ota_ref[h + 1, 4:4 + DH, r0:r1] for h in range(H)], axis=0).astype(BF16)
        r = lax.dot_general(oa, woa_ref[...], TN, preferred_element_type=F32)
        if j == 0:
            o40 = (H // 2 - 1) * 40
            hh_out(_dot(m_ref[H // 2 - 1].astype(BF16), _feat_tile(yt_ref[R_PQ + o40:R_PQ + o40 + 40, :])),
                   o40, 0, S)
        r = r + lax.dot_general(otb_ref[:, r0:r1].astype(BF16), wob_ref[...], TN,
                                preferred_element_type=F32)
        ob_ref[r0:r1, :] = r.astype(BF16)
        ocopy(j).start()
    for j in range(len(OCH)):
        ocopy(j).wait()


@jax.jit
def pallas_gated_mix__mha_block__linear_kernel_hedgehog__prompt_kernel(
    A_x, A_wqkv, A_wo, B_x, B_wqkv, B_w_phi, B_wo, gate_w
):
    x = A_x.reshape(S, D)
    hbm = pl.BlockSpec(memory_space=pl.ANY)
    out = pl.pallas_call(
        _kernel,
        out_shape=jax.ShapeDtypeStruct((S, D), BF16),
        in_specs=[hbm] * 7,
        out_specs=hbm,
        scratch_shapes=[
            pltpu.VMEM((S, D), BF16),
            pltpu.VMEM((D, D), BF16),
            pltpu.VMEM((D, D), BF16),
            pltpu.VMEM((D, D), BF16),
            pltpu.VMEM((D, 3 * D), BF16),
            pltpu.VMEM((D, D), BF16),
            pltpu.VMEM((D, D), BF16),
            pltpu.VMEM((DH, DH, H), BF16),
            pltpu.VMEM((D,), BF16),
            pltpu.VMEM((S, D), BF16),
            pltpu.SemaphoreType.DMA((11,)),
            pltpu.SemaphoreType.DMA((len(OCH),)),
            pltpu.VMEM((R_END, D), BF16),
            pltpu.VMEM((R_END, S), F32),
            pltpu.VMEM((SP, D), BF16),
            pltpu.VMEM((H + 1, 24, S), F32),
            pltpu.VMEM((D, S), F32),
            pltpu.VMEM((D, 128), F32),
            pltpu.VMEM((8, S), F32),
            pltpu.VMEM((2 * D, 128), F32),
            pltpu.VMEM((8, D), F32),
            pltpu.VMEM((H // 2, 48, 80), F32),
            pltpu.VMEM((128, S), BF16),
            pltpu.VMEM((128, 128), BF16),
            pltpu.VMEM((24, S), F32),
            pltpu.VMEM((8, S), F32),
        ],
        compiler_params=pltpu.CompilerParams(vmem_limit_bytes=120 * 1024 * 1024),
    )(x, A_wqkv, A_wo, B_wqkv, jnp.transpose(B_w_phi, (1, 2, 0)), B_wo, gate_w)
    return out.reshape(1, S, D)
```

```python
import functools
import jax
import jax.numpy as jnp
from jax import lax
from jax.experimental import pallas as pl
from jax.experimental.pallas import tpu as pltpu

S, D, H, DH = 2048, 640, 32, 20
LOG2E = 1.4426950408889634
QSCALE = (DH ** -0.5) * LOG2E
F32, BF16 = jnp.float32, jnp.bfloat16
NT = (((1,), (1,)), ((), ()))
TN = (((0,), (0,)), ((), ()))
R_QA, R_VA, R_PQ, R_PK, R_VB, R_G, R_END = 0, 640, 1280, 1920, 2560, 3200, 3216
KT, NKT = 108, 19
SP = 2080
VP = 2176
VROUNDS = (6, 10, 14, 18)
KM = 92
OCH = ((0, 512), (512, 1024), (1024, 1536), (1536, 1920), (1920, 2048))
HS = S // 2
SCORE_LIMIT = 56.0
V_LO, V_HI = 2.0 ** -36, 2.0 ** 50


def _iota(shape, dim):
    return lax.broadcasted_iota(jnp.int32, shape, dim)


def _dot(a, b):
    return jnp.dot(a, b, preferred_element_type=F32)


def _dot_nt(a, b):
    return lax.dot_general(a, b, NT, preferred_element_type=F32)


def _feat_tile(x, seed=None):
    L = x.shape[1]
    x3 = x.reshape(5, 8, L)

    def allred(v, op):
        v = op(v, pltpu.roll(v, 2, 0))
        return op(v, pltpu.roll(v, 4, 0))
    mx = jnp.max(x3, axis=0)
    mn = jnp.min(x3, axis=0)
    if seed is not None:
        mx = mx + seed
        mn = mn + seed
    mx = allred(mx, jnp.maximum)
    mn = allred(mn, jnp.minimum)
    ep = jnp.exp2(x3 - mx[None])
    en = jnp.exp2(mn[None] - x3)
    rp = 1.0 / allred(jnp.sum(ep, axis=0), jnp.add)
    rn = 1.0 / allred(jnp.sum(en, axis=0), jnp.add)
    return jnp.concatenate([(ep * rp[None]).reshape(40, L), (en * rn[None]).reshape(40, L)],
                           axis=0).astype(BF16)


def _kernel(x_hbm, wa_hbm, woa_hbm, wb_hbm, phi_hbm, wob_hbm, gate_hbm, out_hbm,
            x_ref, wq_ref, wk_ref, wv_ref, wb_ref, woa_ref, wob_ref, phi_ref, gate_ref, ob_ref, sems, osems,
            wt_ref, yt_ref, ks_ref, ota_ref, otb_ref,
            phi2_ref, g_ref, am_ref, km_ref, m_ref, w0_ref, l0_ref, ao_ref, al_ref, qf_ref, kb_ref):
    X0, X1 = 512, 1792

    def xcopy(r0, r1, k):
        return pltpu.make_async_copy(x_hbm.at[pl.ds(r0, r1 - r0), :], x_ref.at[pl.ds(r0, r1 - r0), :], sems.at[k])
    c_wk = pltpu.make_async_copy(wa_hbm.at[:, pl.ds(D, D)], wk_ref, sems.at[0])
    c_x0 = xcopy(0, X0, 1)
    c_x1 = xcopy(X0, X1, 2)
    c_phi = pltpu.make_async_copy(phi_hbm, phi_ref, sems.at[3])
    c_gate = pltpu.make_async_copy(gate_hbm, gate_ref, sems.at[4])
    c_wq = pltpu.make_async_copy(wa_hbm.at[:, pl.ds(0, D)], wq_ref, sems.at[5])
    c_wv = pltpu.make_async_copy(wa_hbm.at[:, pl.ds(2 * D, D)], wv_ref, sems.at[6])
    c_wb = pltpu.make_async_copy(wb_hbm, wb_ref, sems.at[7])
    c_x2 = xcopy(X1, S, 8)
    c_woa = pltpu.make_async_copy(woa_hbm, woa_ref, sems.at[9])
    c_wob = pltpu.make_async_copy(wob_hbm, wob_ref, sems.at[10])
    for c in (c_wk, c_x0, c_x1, c_phi, c_gate, c_wq, c_wv, c_wb, c_x2, c_woa, c_wob):
        c.start()

    def proj_k(r0, n):
        km = None
        for q in range(4):
            a, b = r0 + q * n // 4, r0 + (q + 1) * n // 4
            k = _dot(x_ref[a:b, :], wk_ref[...])
            ks_ref[a:b, :] = k.astype(BF16)
            m = jnp.max(jnp.abs(k).reshape((b - a) // 8, 8, D), axis=0)
            km = m if km is None else jnp.maximum(km, m)
        return km
    ks_ref[S:SP, :] = jnp.zeros((SP - S, D), BF16)
    c_wk.wait()
    c_x0.wait()
    km = proj_k(0, X0)
    c_x1.wait()
    km = jnp.maximum(km, proj_k(X0, X1 - X0))
    for c in (c_phi, c_gate, c_wq, c_wv, c_wb, c_x2):
        c.wait()
    km_ref[...] = jnp.maximum(km, proj_k(X1, S - X1))

    for d in range(DH):
        pt = phi_ref[d].astype(F32).T
        phi2_ref[pl.ds(d, H, stride=DH), :] = jnp.concatenate(
            [pt, jnp.zeros((H, 128 - DH), F32)], axis=1)

    wt_ref[R_QA:R_QA + D, :] = wq_ref[...].T
    wt_ref[R_VA:R_VA + D, :] = wv_ref[...].T
    wt_ref[R_VB:R_VB + D, :] = wb_ref[:, 2 * D:3 * D].T
    grow = jnp.broadcast_to(gate_ref[...].astype(F32).reshape(1, D), (16, D))
    wt_ref[R_G:R_END, :] = jnp.where(_iota((16, D), 0) == 0, grow, 0.0).astype(BF16)

    ri = _iota((128, 128), 0)
    ci = _iota((128, 128), 1)
    sel = ((ri % 40) // 2 == ci).astype(BF16)
    keep = (2 * (ri // 40) + ri % 2 == ci // DH) & (ri < 120)
    for g in range(6):
        n = 120 if g < 5 else 40
        c0 = min(120 * g, D - 128)
        pw = phi2_ref[c0:c0 + 128, :].astype(BF16)
        rep = _dot_nt(sel, pw)
        if g < 5:
            kp = keep
        else:
            kp = (30 + 2 * (ri // 40) + ri % 2 == (c0 + ci) // DH) & (ri < 40)
        lg = jnp.where(kp, rep, 0.0).astype(BF16)
        for col0, r0 in ((0, R_PQ), (D, R_PK)):
            fold = _dot_nt(lg, wb_ref[:, col0 + c0:col0 + c0 + 128]) * LOG2E
            yt_ref[r0 - R_PQ + 120 * g:r0 - R_PQ + 120 * g + n, 0:D] = fold[0:n]
    wt_ref[R_PQ:R_VB, :] = yt_ref[0:2 * D, 0:D].astype(BF16)

    PC = 256

    def proj_t(j, c):
        off = pl.multiple_of(j * PC, PC)
        y = _dot_nt(wt_ref[...], x_ref[pl.ds(off, PC), :])
        yt_ref[:, pl.ds(off, PC)] = y
        ay = jnp.abs(y[0:2 * D])
        am = jnp.maximum(ay[:, 0:128], ay[:, 128:256])
        am_ref[...] = jnp.maximum(am, am_ref[...])
        return c
    am_ref[...] = jnp.zeros(am_ref.shape, F32)
    lax.fori_loop(0, S // PC, proj_t, 0)

    kmax = jnp.max(km_ref[...], axis=0, keepdims=True)
    seg = _iota((H, D), 1) // DH == _iota((H, D), 0)
    amat = jnp.where(seg, jnp.broadcast_to(kmax, (H, D)), 0.0).astype(BF16)
    bound = jnp.max(_dot(amat, (am_ref[R_QA:R_QA + D, :] * QSCALE).astype(BF16)))
    vmax = jnp.max(am_ref[R_VA:R_VA + D, :])
    safe = (bound <= SCORE_LIMIT) & (vmax >= V_LO) & (vmax <= V_HI)

    g_ref[...] = jnp.broadcast_to(jax.nn.sigmoid(yt_ref[R_G:R_G + 1, :]), (8, S))

    mr = _iota((48, 80), 0)
    mkeep = jnp.where(mr < 40, mr // DH, mr - 40) == _iota((48, 80), 1) % 2

    def hh_lv(o40, c0, n):
        ones8 = jnp.where(_iota((8, n), 0) < 2, 1.0, 0.0)
        return jnp.concatenate([yt_ref[pl.ds(R_VB + o40, 40), pl.ds(c0, n)], ones8], axis=0).astype(BF16)

    def hh_out(nd, o40, c0, n):
        omg = 1.0 - g_ref[0:1, pl.ds(c0, n)]
        s0 = omg / (nd[40:41, :] + 1e-6)
        s1 = omg / (nd[41:42, :] + 1e-6)
        otb_ref[pl.ds(o40, 40), pl.ds(c0, n)] = nd[0:40, :] * jnp.where(_iota((40, n), 0) < DH, s0, s1)

    def head_rows(r0, hd):
        lo = hd * DH
        w32 = yt_ref[pl.ds(pl.multiple_of(r0 + (lo // 8) * 8, 8), 32), :]
        return jnp.where(hd % 2 == 1, w32[4:28], w32[0:24])

    def head_geom(h):
        lo = h * DH
        a = lo // 128
        return (pl.multiple_of(a * 128, 128), pl.multiple_of(jnp.minimum(a + 1, 4) * 128, 128),
                lo - a * 128)

    @pl.when(safe)
    def _fast():
        sub8 = _iota((8, S), 0)
        lane = _iota((1, 128), 1)

        def q_rows(hd):
            qf = head_rows(R_QA, hd) * QSCALE
            return pltpu.roll(qf[0:8], 4, 0), qf[4:20], qf

        def v_rows(hd):
            return jnp.concatenate([head_rows(R_VA, hd)[0:DH], jnp.zeros((DH, VP - S), F32)], axis=1)

        def k_part(hk, tk, seed=None):
            ca, cb, off = head_geom(hk)
            r0 = (KT * tk) // 16 * 16
            o = KT * tk - r0
            ka = ks_ref[r0:r0 + 128, pl.ds(ca, 128)].astype(F32)[o:o + KT]
            kb = ks_ref[r0:r0 + 128, pl.ds(cb, 128)].astype(F32)[o:o + KT]
            kp = jnp.where(lane >= off, ka, kb)
            if seed is not None:
                kp = kp + seed
            kp = pltpu.roll(kp, (KT + 128 - off) % 128, 1)
            return jnp.where(lane >= KT, kp, 0.0)

        def make_lhs(hk, tk, vf, tv, seed=None):
            kp = k_part(hk, tk, seed)
            if tk in VROUNDS:
                kp = kp[0:KM]
            if vf is not None:
                vp = jnp.where(lane < KT, vf[:, KT * tv:KT * tv + 128], 0.0)
            else:
                vp = jnp.zeros((DH, 128), F32)
            return jnp.concatenate([kp, vp], axis=0).astype(BF16)

        def build_kb(hk, tk, seed=None):
            ca, cb, off = head_geom(hk)
            r0 = (KT * tk + KM) // 16 * 16
            o = KT * tk + KM - r0
            ka = ks_ref[r0:r0 + 32, pl.ds(ca, 128)].astype(F32)[o:o + 16]
            kb = ks_ref[r0:r0 + 32, pl.ds(cb, 128)].astype(F32)[o:o + 16]
            kp = jnp.where(lane >= off, ka, kb)
            if seed is not None:
                kp = kp + seed
            kp = pltpu.roll(kp, (128 - off) % 128, 1)
            kp = jnp.concatenate([pltpu.roll(kp[0:8], 4, 0), pltpu.roll(kp[8:16], 4, 0)], axis=0)
            i = VROUNDS.index(tk)
            for d in range(DH):
                kb_ref[i * DH + d] = jnp.broadcast_to(kp[:, d:d + 1], (16, 128))

        def piece(tv, j, seed, kbv):
            a0 = a1 = seed
            for d in range(DH):
                q = qf_ref[d:d + 1, j * 128:(j + 1) * 128]
                a0 = a0 + kbv[d][0:8] * q
                a1 = a1 + kbv[d][8:16] * q
            return jnp.exp2(jnp.concatenate([a0, a1], axis=0))

        todo = [(tv, j) for tv in VROUNDS for j in range(S // 128)]
        plan = {t: [] for t in range(NKT)}
        for n, (tv, j) in enumerate(todo):
            plan[min(int(n * (VROUNDS[-1] - 1) / len(todo)), tv - 2)].append((tv, j))

        def make_w(e, qt, qb):
            return jnp.concatenate([e[0:104], jnp.where(sub8 < 4, e[104:112], qt), qb], axis=0).astype(BF16)

        def fin(ao, al, slot):
            inv = g_ref[0:1, :] / jnp.sum(al, axis=0, keepdims=True)
            ota_ref[slot] = ao * inv

        qt0, qb0, _ = q_rows(0)
        for tv in VROUNDS:
            build_kb(0, tv)
        w0_ref[...] = make_w(jnp.zeros((112, S), F32), qt0, qb0)
        l0_ref[...] = make_lhs(0, 0, None, 0)
        ao_ref[...] = jnp.zeros(ao_ref.shape, F32)
        al_ref[...] = jnp.ones(al_ref.shape, F32)
        m_ref[...] = jnp.zeros(m_ref.shape, F32)

        def head(h, c):
            hn = jnp.minimum(h + 1, H - 1)
            qt, qb, qf = q_rows(h)
            qf_ref[...] = qf
            pieces = {}
            ties = {t: [] for t in range(NKT + 2)}
            vf = v_rows(h)
            pk = h // 2
            pq = jnp.maximum(pk - 1, 0)
            c0 = pl.multiple_of((h % 2) * HS, HS)
            ok = pl.multiple_of(pk * 40, 8)
            oq = pl.multiple_of(pq * 40, 8)
            fq, fk = [], []
            w = w0_ref[...]
            lhs = l0_ref[...]
            ao, al = ao_ref[...], al_ref[...]
            prev = None
            for t in range(NKT):
                out = _dot(lhs, w)
                seed = None if prev is None else prev[0:8, 0:128] * 0.0
                useed = None if seed is None else seed[0:1]
                if t + 1 < NKT:
                    lhs = make_lhs(h, t + 1, vf, t, useed)
                else:
                    lhs = make_lhs(hn, 0, vf, t, useed)
                if t in VROUNDS:
                    ao = ao + out[88:112]
                else:
                    ao = ao + out[104:128]
                if t == 0:
                    fin(ao, al, h)
                    ao = jnp.zeros((24, S), F32)
                    al = None
                if t in VROUNDS:
                    ev = jnp.concatenate([pieces.pop((t, j)) for j in range(S // 128)], axis=1)
                    em = jnp.exp2(out[0:96])
                    xr, yr = ev[0:8], ev[8:16]
                    e = jnp.concatenate([em[0:88], jnp.where(sub8 < 4, em[88:96], xr),
                                         jnp.where(sub8 < 4, xr, yr), yr], axis=0)
                    build_kb(hn, t, out[0:1, 128:256] * 0.0)
                else:
                    e = jnp.exp2(out[0:112])
                if ties[t]:
                    top = [e[0:8, 128 * j:128 * (j + 1)] for j in range(S // 128)]
                    for n, v in enumerate(ties[t]):
                        j = (n * (S // 128)) // len(ties[t])
                        top[j] = top[j] + v
                    e = jnp.concatenate([jnp.concatenate(top, axis=1), e[8:112]], axis=0)
                kbs = {tv: [kb_ref[VROUNDS.index(tv) * DH + d] for d in range(DH)] for tv in set(p[0] for p in plan[t])}
                for n, (tv, j) in enumerate(plan[t]):
                    r, cq = (16 * n) % 88, ((n * 16) // max(len(plan[t]), 1)) * 128
                    pieces[(tv, j)] = piece(tv, j, out[r:r + 8, cq:cq + 128] * 0.0, kbs[tv])
                    if t + 1 < tv:
                        ties[t + 1].append(pieces[(tv, j)][0:8] * 0.0)
                last = e[104:112]
                last = jnp.where(sub8 < (4 if t + 1 < NKT else 0), last, 0.0)
                tot = functools.reduce(jnp.add, [e[8 * i:8 * i + 8] for i in range(13)] + [last])
                al = tot if al is None else al + tot
                if t + 1 < NKT:
                    w = make_w(e, qt, qb)
                else:
                    w = make_w(e, *q_rows(hn)[0:2])
                if seed is not None and t <= 8:
                    u = len(fq)
                    fq.append(_feat_tile(yt_ref[pl.ds(R_PQ + oq, 40), pl.ds(c0 + 128 * u, 128)], seed))
                    ties[t + 1].append(fq[-1][0:16].astype(F32)[0:8] * 0.0)
                elif 9 <= t <= 16:
                    u = len(fk)
                    fk.append(_feat_tile(yt_ref[pl.ds(R_PK + ok, 40), pl.ds(c0 + 128 * u, 128)], seed))
                    ties[t + 1].append(fk[-1][0:16].astype(F32)[0:8] * 0.0)
                prev = out
            hh_out(_dot(m_ref[pq].astype(BF16), jnp.concatenate(fq, axis=1)), oq, c0, HS)
            kv = _dot_nt(hh_lv(ok, c0, HS), jnp.concatenate(fk, axis=1))
            kv = jnp.where(mkeep, kv, 0.0)
            m_ref[pk] = jnp.where(h % 2 == 0, kv, kv + m_ref[pk])
            w0_ref[...] = w
            l0_ref[...] = lhs
            ao_ref[...] = ao
            al_ref[...] = al
            return c
        lax.fori_loop(0, H, head, 0)
        out = _dot(l0_ref[...], w0_ref[...])
        fin(ao_ref[...] + out[104:128], al_ref[...], H)

    @pl.when(jnp.logical_not(safe))
    def _slow():
        def pair(p, c):
            o40 = pl.multiple_of(p * 40, 8)
            kv = _dot_nt(hh_lv(o40, 0, S), _feat_tile(yt_ref[pl.ds(R_PK + o40, 40), :]))
            m = jnp.where(mkeep, kv, 0.0)
            m_ref[p] = m
            hh_out(_dot(m.astype(BF16), _feat_tile(yt_ref[pl.ds(R_PQ + o40, 40), :])), o40, 0, S)
            return c
        lax.fori_loop(0, H // 2, pair, 0)

        def slow(i, c):
            h = i // (S // 256)
            c0 = pl.multiple_of((i % (S // 256)) * 256, 256)
            ca, cb, off = head_geom(h)
            s = None
            for cw, first in ((ca, True), (cb, False)):
                rows = _iota((128, 256), 0) + (0 if first else 128)
                msk = (rows >= off) & (rows < off + DH)
                if not first:
                    msk = msk & (cb != ca)
                qm = jnp.where(msk, yt_ref[pl.ds(cw, 128), pl.ds(c0, 256)] * QSCALE, 0.0).astype(BF16)
                part = _dot(ks_ref[0:S, pl.ds(cw, 128)], qm)
                s = part if s is None else s + part
            p = jnp.exp2(s - jnp.max(s, axis=0, keepdims=True)).astype(BF16)
            vf = head_rows(R_VA, h)[0:DH]
            c256 = jnp.concatenate([vf, jnp.where(_iota((12, S), 0) == 0, 1.0, 0.0)], axis=0).astype(BF16)
            o = _dot(c256, p)
            o = jnp.concatenate([o[28:32], o[0:DH]], axis=0) * (g_ref[0:1, pl.ds(c0, 256)] / o[DH:DH + 1])
            ota_ref[h + 1, :, pl.ds(c0, 256)] = o
            return c
        lax.fori_loop(0, H * (S // 256), slow, 0)

    c_woa.wait()
    c_wob.wait()

    def ocopy(j):
        r0, r1 = OCH[j]
        return pltpu.make_async_copy(ob_ref.at[pl.ds(r0, r1 - r0), :],
                                     out_hbm.at[pl.ds(r0, r1 - r0), :], osems.at[j])

    for j, (r0, r1) in enumerate(OCH):
        oa = jnp.concatenate([ota_ref[h + 1, 4:4 + DH, r0:r1] for h in range(H)], axis=0).astype(BF16)
        r = lax.dot_general(oa, woa_ref[...], TN, preferred_element_type=F32)
        if j == 0:
            o40 = (H // 2 - 1) * 40
            hh_out(_dot(m_ref[H // 2 - 1].astype(BF16), _feat_tile(yt_ref[R_PQ + o40:R_PQ + o40 + 40, :])),
                   o40, 0, S)
        r = r + lax.dot_general(otb_ref[:, r0:r1].astype(BF16), wob_ref[...], TN,
                                preferred_element_type=F32)
        ob_ref[r0:r1, :] = r.astype(BF16)
        ocopy(j).start()
    for j in range(len(OCH)):
        ocopy(j).wait()


@jax.jit
def pallas_gated_mix__mha_block__linear_kernel_hedgehog__prompt_kernel(
    A_x, A_wqkv, A_wo, B_x, B_wqkv, B_w_phi, B_wo, gate_w
):
    x = A_x.reshape(S, D)
    hbm = pl.BlockSpec(memory_space=pl.ANY)
    out = pl.pallas_call(
        _kernel,
        out_shape=jax.ShapeDtypeStruct((S, D), BF16),
        in_specs=[hbm] * 7,
        out_specs=hbm,
        scratch_shapes=[
            pltpu.VMEM((S, D), BF16),
            pltpu.VMEM((D, D), BF16),
            pltpu.VMEM((D, D), BF16),
            pltpu.VMEM((D, D), BF16),
            pltpu.VMEM((D, 3 * D), BF16),
            pltpu.VMEM((D, D), BF16),
            pltpu.VMEM((D, D), BF16),
            pltpu.VMEM((DH, DH, H), BF16),
            pltpu.VMEM((D,), BF16),
            pltpu.VMEM((S, D), BF16),
            pltpu.SemaphoreType.DMA((11,)),
            pltpu.SemaphoreType.DMA((len(OCH),)),
            pltpu.VMEM((R_END, D), BF16),
            pltpu.VMEM((R_END, S), F32),
            pltpu.VMEM((SP, D), BF16),
            pltpu.VMEM((H + 1, 24, S), F32),
            pltpu.VMEM((D, S), F32),
            pltpu.VMEM((D, 128), F32),
            pltpu.VMEM((8, S), F32),
            pltpu.VMEM((2 * D, 128), F32),
            pltpu.VMEM((8, D), F32),
            pltpu.VMEM((H // 2, 48, 80), F32),
            pltpu.VMEM((128, S), BF16),
            pltpu.VMEM((128, 128), BF16),
            pltpu.VMEM((24, S), F32),
            pltpu.VMEM((8, S), F32),
            pltpu.VMEM((24, S), F32),
            pltpu.VMEM((len(VROUNDS) * DH, 16, 128), F32),
        ],
        compiler_params=pltpu.CompilerParams(vmem_limit_bytes=120 * 1024 * 1024),
    )(x, A_wqkv, A_wo, B_wqkv, jnp.transpose(B_w_phi, (1, 2, 0)), B_wo, gate_w)
    return out.reshape(1, S, D)
```

```python
import functools
import jax
import jax.numpy as jnp
from jax import lax
from jax.experimental import pallas as pl
from jax.experimental.pallas import tpu as pltpu

S, D, H, DH = 2048, 640, 32, 20
LOG2E = 1.4426950408889634
QSCALE = (DH ** -0.5) * LOG2E
F32, BF16 = jnp.float32, jnp.bfloat16
NT = (((1,), (1,)), ((), ()))
TN = (((0,), (0,)), ((), ()))
R_QA, R_VA, R_PQ, R_PK, R_VB, R_G, R_END = 0, 640, 1280, 1920, 2560, 3200, 3216
KT, NKT = 108, 19
SP = 2080
VP = 2176
VROUNDS = (6, 10, 14, 17)
KM = 92
OCH = ((0, 512), (512, 1024), (1024, 1536), (1536, 1920), (1920, 2048))
HS = S // 2
SCORE_LIMIT = 56.0
V_LO, V_HI = 2.0 ** -36, 2.0 ** 50


def _iota(shape, dim):
    return lax.broadcasted_iota(jnp.int32, shape, dim)


def _dot(a, b):
    return jnp.dot(a, b, preferred_element_type=F32)


def _dot_nt(a, b):
    return lax.dot_general(a, b, NT, preferred_element_type=F32)


def _feat_tile(x, seed=None):
    L = x.shape[1]
    x3 = x.reshape(5, 8, L)

    def allred(v, op):
        v = op(v, pltpu.roll(v, 2, 0))
        return op(v, pltpu.roll(v, 4, 0))
    mx = jnp.max(x3, axis=0)
    mn = jnp.min(x3, axis=0)
    if seed is not None:
        mx = mx + seed
        mn = mn + seed
    mx = allred(mx, jnp.maximum)
    mn = allred(mn, jnp.minimum)
    ep = jnp.exp2(x3 - mx[None])
    en = jnp.exp2(mn[None] - x3)
    rp = 1.0 / allred(jnp.sum(ep, axis=0), jnp.add)
    rn = 1.0 / allred(jnp.sum(en, axis=0), jnp.add)
    return jnp.concatenate([(ep * rp[None]).reshape(40, L), (en * rn[None]).reshape(40, L)],
                           axis=0).astype(BF16)


def _kernel(x_hbm, wa_hbm, woa_hbm, wb_hbm, phi_hbm, wob_hbm, gate_hbm, out_hbm,
            x_ref, wq_ref, wk_ref, wv_ref, wb_ref, woa_ref, wob_ref, phi_ref, gate_ref, ob_ref, sems, osems,
            wt_ref, yt_ref, ks_ref, ota_ref, otb_ref,
            phi2_ref, g_ref, am_ref, km_ref, m_ref, w0_ref, l0_ref, ao_ref, al_ref, qf_ref, kb_ref):
    X0, X1 = 512, 1280

    def xcopy(r0, r1, k):
        return pltpu.make_async_copy(x_hbm.at[pl.ds(r0, r1 - r0), :], x_ref.at[pl.ds(r0, r1 - r0), :], sems.at[k])
    c_wk = pltpu.make_async_copy(wa_hbm.at[:, pl.ds(D, D)], wk_ref, sems.at[0])
    c_x0 = xcopy(0, X0, 1)
    c_x1 = xcopy(X0, X1, 2)
    c_phi = pltpu.make_async_copy(phi_hbm, phi_ref, sems.at[3])
    c_gate = pltpu.make_async_copy(gate_hbm, gate_ref, sems.at[4])
    c_wq = pltpu.make_async_copy(wa_hbm.at[:, pl.ds(0, D)], wq_ref, sems.at[5])
    c_wv = pltpu.make_async_copy(wa_hbm.at[:, pl.ds(2 * D, D)], wv_ref, sems.at[6])
    c_wb = pltpu.make_async_copy(wb_hbm, wb_ref, sems.at[7])
    c_x2 = xcopy(X1, S, 8)
    c_woa = pltpu.make_async_copy(woa_hbm, woa_ref, sems.at[9])
    c_wob = pltpu.make_async_copy(wob_hbm, wob_ref, sems.at[10])
    for c in (c_wk, c_x0, c_x1, c_phi, c_gate, c_wq, c_wv, c_x2, c_wb, c_woa, c_wob):
        c.start()

    def proj_k(r0, n):
        km = None
        for q in range(4):
            a, b = r0 + q * n // 4, r0 + (q + 1) * n // 4
            k = _dot(x_ref[a:b, :], wk_ref[...])
            ks_ref[a:b, :] = k.astype(BF16)
            m = jnp.max(jnp.abs(k).reshape((b - a) // 8, 8, D), axis=0)
            km = m if km is None else jnp.maximum(km, m)
        return km
    ks_ref[S:SP, :] = jnp.zeros((SP - S, D), BF16)
    w0_ref[0:96, :] = jnp.zeros((96, S), BF16)
    ao_ref[...] = jnp.zeros(ao_ref.shape, F32)
    al_ref[...] = jnp.ones(al_ref.shape, F32)
    m_ref[...] = jnp.zeros(m_ref.shape, F32)
    am_ref[...] = jnp.zeros(am_ref.shape, F32)
    c_wk.wait()
    c_x0.wait()
    km = proj_k(0, X0)
    c_x1.wait()
    km = jnp.maximum(km, proj_k(X0, X1 - X0))
    for c in (c_phi, c_gate, c_wq, c_wv, c_x2):
        c.wait()
    km_ref[...] = jnp.maximum(km, proj_k(X1, S - X1))

    for d in range(DH):
        pt = phi_ref[d].astype(F32).T
        phi2_ref[pl.ds(d, H, stride=DH), :] = jnp.concatenate(
            [pt, jnp.zeros((H, 128 - DH), F32)], axis=1)

    wt_ref[R_QA:R_QA + D, :] = wq_ref[...].T
    wt_ref[R_VA:R_VA + D, :] = wv_ref[...].T
    grow = jnp.broadcast_to(gate_ref[...].astype(F32).reshape(1, D), (16, D))
    wt_ref[R_G:R_END, :] = jnp.where(_iota((16, D), 0) == 0, grow, 0.0).astype(BF16)

    c_wb.wait()
    wt_ref[R_VB:R_VB + D, :] = wb_ref[:, 2 * D:3 * D].T

    ri = _iota((128, 128), 0)
    ci = _iota((128, 128), 1)
    sel = ((ri % 40) // 2 == ci).astype(BF16)
    keep = (2 * (ri // 40) + ri % 2 == ci // DH) & (ri < 120)
    for g in range(6):
        n = 120 if g < 5 else 40
        c0 = min(120 * g, D - 128)
        pw = phi2_ref[c0:c0 + 128, :].astype(BF16)
        rep = _dot_nt(sel, pw)
        if g < 5:
            kp = keep
        else:
            kp = (30 + 2 * (ri // 40) + ri % 2 == (c0 + ci) // DH) & (ri < 40)
        lg = jnp.where(kp, rep, 0.0).astype(BF16)[0:(128 if g < 5 else 48)]
        for col0, r0 in ((0, R_PQ), (D, R_PK)):
            fold = _dot_nt(lg, wb_ref[:, col0 + c0:col0 + c0 + 128]) * LOG2E
            yt_ref[r0 - R_PQ + 120 * g:r0 - R_PQ + 120 * g + n, 0:D] = fold[0:n]
    wt_ref[R_PQ:R_VB, :] = yt_ref[0:2 * D, 0:D].astype(BF16)

    def head_rows(r0, hd):
        lo = hd * DH
        w32 = yt_ref[pl.ds(pl.multiple_of(r0 + (lo // 8) * 8, 8), 32), :]
        return jnp.where(hd % 2 == 1, w32[4:28], w32[0:24])

    def head_geom(h):
        lo = h * DH
        a = lo // 128
        return (pl.multiple_of(a * 128, 128), pl.multiple_of(jnp.minimum(a + 1, 4) * 128, 128),
                lo - a * 128)

    sub8 = _iota((8, S), 0)
    lane = _iota((1, 128), 1)

    def q_rows(hd):
        qf = head_rows(R_QA, hd) * QSCALE
        return pltpu.roll(qf[0:8], 4, 0), qf[4:20], qf

    def v_rows(hd):
        return jnp.concatenate([head_rows(R_VA, hd)[0:DH], jnp.zeros((DH, VP - S), F32)], axis=1)

    def k_part(hk, tk, seed=None):
        ca, cb, off = head_geom(hk)
        r0 = (KT * tk) // 16 * 16
        o = KT * tk - r0
        ka = ks_ref[r0:r0 + 128, pl.ds(ca, 128)].astype(F32)[o:o + KT]
        kb = ks_ref[r0:r0 + 128, pl.ds(cb, 128)].astype(F32)[o:o + KT]
        kp = jnp.where(lane >= off, ka, kb)
        if seed is not None:
            kp = kp + seed
        kp = pltpu.roll(kp, (KT + 128 - off) % 128, 1)
        return jnp.where(lane >= KT, kp, 0.0)

    def make_lhs(hk, tk, vf, tv, seed=None):
        kp = k_part(hk, tk, seed)
        if tk in VROUNDS:
            kp = kp[0:KM]
        if vf is not None:
            vp = jnp.where(lane < KT, vf[:, KT * tv:KT * tv + 128], 0.0)
        else:
            vp = jnp.zeros((DH, 128), F32)
        return jnp.concatenate([kp, vp], axis=0).astype(BF16)

    def build_kb(hk, tk, seed=None):
        ca, cb, off = head_geom(hk)
        r0 = (KT * tk + KM) // 16 * 16
        o = KT * tk + KM - r0
        ka = ks_ref[r0:r0 + 32, pl.ds(ca, 128)].astype(F32)[o:o + 16]
        kb = ks_ref[r0:r0 + 32, pl.ds(cb, 128)].astype(F32)[o:o + 16]
        kp = jnp.where(lane >= off, ka, kb)
        if seed is not None:
            kp = kp + seed
        kp = pltpu.roll(kp, (128 - off) % 128, 1)
        kp = jnp.concatenate([pltpu.roll(kp[0:8], 4, 0), pltpu.roll(kp[8:16], 4, 0)], axis=0)
        i = VROUNDS.index(tk)
        for d in range(DH):
            kb_ref[i * DH + d] = jnp.broadcast_to(kp[:, d:d + 1], (16, 128))

    for tv in VROUNDS:
        build_kb(0, tv)
    l0_ref[...] = make_lhs(0, 0, None, 0)

    PC = 256

    def proj_t(j, c):
        off = pl.multiple_of(j * PC, PC)
        y = _dot_nt(wt_ref[...], x_ref[pl.ds(off, PC), :])
        yt_ref[:, pl.ds(off, PC)] = y
        ay = jnp.abs(y[0:2 * D])
        am = jnp.maximum(ay[:, 0:128], ay[:, 128:256])
        am_ref[...] = jnp.maximum(am, am_ref[...])
        return c
    lax.fori_loop(0, S // PC, proj_t, 0)

    kmax = jnp.max(km_ref[...], axis=0, keepdims=True)
    seg = _iota((H, D), 1) // DH == _iota((H, D), 0)
    amat = jnp.where(seg, jnp.broadcast_to(kmax, (H, D)), 0.0).astype(BF16)
    bound = jnp.max(_dot(amat, (am_ref[R_QA:R_QA + D, :] * QSCALE).astype(BF16)))
    vmax = jnp.max(am_ref[R_VA:R_VA + D, :])
    safe = (bound <= SCORE_LIMIT) & (vmax >= V_LO) & (vmax <= V_HI)

    g_ref[...] = jnp.broadcast_to(jax.nn.sigmoid(yt_ref[R_G:R_G + 1, :]), (8, S))

    mr = _iota((48, 80), 0)
    mkeep = jnp.where(mr < 40, mr // DH, mr - 40) == _iota((48, 80), 1) % 2

    def hh_lv(o40, c0, n):
        ones8 = jnp.where(_iota((8, n), 0) < 2, 1.0, 0.0)
        return jnp.concatenate([yt_ref[pl.ds(R_VB + o40, 40), pl.ds(c0, n)], ones8], axis=0).astype(BF16)

    def hh_out(nd, o40, c0, n):
        omg = 1.0 - g_ref[0:1, pl.ds(c0, n)]
        s0 = omg / (nd[40:41, :] + 1e-6)
        s1 = omg / (nd[41:42, :] + 1e-6)
        otb_ref[pl.ds(o40, 40), pl.ds(c0, n)] = nd[0:40, :] * jnp.where(_iota((40, n), 0) < DH, s0, s1)

    def piece(tv, j, seed, kbv):
        a0 = a1 = seed
        for d in range(DH):
            q = qf_ref[d, :, j * 128:(j + 1) * 128]
            a0 = a0 + kbv[d][0:8] * q
            a1 = a1 + kbv[d][8:16] * q
        return jnp.exp2(jnp.concatenate([a0, a1], axis=0))

    todo = [(tv, j) for tv in VROUNDS for j in range(S // 128)]
    plan = {t: [] for t in range(NKT)}
    for n, (tv, j) in enumerate(todo):
        plan[min(int(n * (VROUNDS[-1] - 1) / len(todo)), tv - 2)].append((tv, j))

    def make_w(e, qt, qb):
        return jnp.concatenate([e[0:104], jnp.where(sub8 < 4, e[104:112], qt), qb], axis=0).astype(BF16)

    def fin(ao, al, slot):
        inv = g_ref[0:1, :] / jnp.sum(al, axis=0, keepdims=True)
        ota_ref[slot] = ao * inv

    qt0, qb0, _ = q_rows(0)
    w0_ref[96:128, :] = make_w(jnp.zeros((112, S), F32), qt0, qb0)[96:128]

    @pl.when(safe)
    def _fast():
        def head(h, c):
            hn = jnp.minimum(h + 1, H - 1)
            qt, qb, qf = q_rows(h)
            for d in range(DH):
                qf_ref[d] = jnp.broadcast_to(qf[d:d + 1], (8, S))
            pieces = {}
            ties = {t: [] for t in range(NKT + 2)}
            vf = v_rows(h)
            pk = h // 2
            pq = jnp.maximum(pk - 1, 0)
            c0 = pl.multiple_of((h % 2) * HS, HS)
            ok = pl.multiple_of(pk * 40, 8)
            oq = pl.multiple_of(pq * 40, 8)
            fq, fk = [], []
            w = w0_ref[...]
            lhs = l0_ref[...]
            ao, al = ao_ref[...], al_ref[...]
            prev = None
            for t in range(NKT):
                out = _dot(lhs, w)
                seed = None if prev is None else prev[0:8, 0:128] * 0.0
                useed = None if seed is None else seed[0:1]
                if t + 1 < NKT:
                    lhs = make_lhs(h, t + 1, vf, t, useed)
                else:
                    lhs = make_lhs(hn, 0, vf, t, useed)
                if t in VROUNDS:
                    ao = ao + out[88:112]
                else:
                    ao = ao + out[104:128]
                if t == 0:
                    fin(ao, al, h)
                    ao = jnp.zeros((24, S), F32)
                    al = None
                if t in VROUNDS:
                    ev = jnp.concatenate([pieces.pop((t, j)) for j in range(S // 128)], axis=1)
                    em = jnp.exp2(out[0:96])
                    xr, yr = ev[0:8], ev[8:16]
                    e = jnp.concatenate([em[0:88], jnp.where(sub8 < 4, em[88:96], xr),
                                         jnp.where(sub8 < 4, xr, yr), yr], axis=0)
                    build_kb(hn, t, out[0:1, 128:256] * 0.0)
                else:
                    e = jnp.exp2(out[0:112])
                if ties[t]:
                    top = [e[0:8, 128 * j:128 * (j + 1)] for j in range(S // 128)]
                    for n, v in enumerate(ties[t]):
                        j = (n * (S // 128)) // len(ties[t])
                        top[j] = top[j] + v
                    e = jnp.concatenate([jnp.concatenate(top, axis=1), e[8:112]], axis=0)
                kbs = {tv: [kb_ref[VROUNDS.index(tv) * DH + d] for d in range(DH)] for tv in set(p[0] for p in plan[t])}
                for n, (tv, j) in enumerate(plan[t]):
                    r, cq = (16 * n) % 88, ((n * 16) // max(len(plan[t]), 1)) * 128
                    pieces[(tv, j)] = piece(tv, j, out[r:r + 8, cq:cq + 128] * 0.0, kbs[tv])
                    if t + 1 < tv:
                        ties[t + 1].append(pieces[(tv, j)][0:8] * 0.0)
                last = e[104:112]
                last = jnp.where(sub8 < (4 if t + 1 < NKT else 0), last, 0.0)
                tot = functools.reduce(jnp.add, [e[8 * i:8 * i + 8] for i in range(13)] + [last])
                al = tot if al is None else al + tot
                if t + 1 < NKT:
                    w = make_w(e, qt, qb)
                else:
                    w = make_w(e, *q_rows(hn)[0:2])
                if 2 <= t < 10:
                    u = len(fq)
                    fq.append(_feat_tile(yt_ref[pl.ds(R_PQ + oq, 40), pl.ds(c0 + 128 * u, 128)], seed))
                    ties[t + 1].append(fq[-1][0:16].astype(F32)[0:8] * 0.0)
                elif 10 <= t < 18:
                    u = len(fk)
                    fk.append(_feat_tile(yt_ref[pl.ds(R_PK + ok, 40), pl.ds(c0 + 128 * u, 128)], seed))
                    ties[t + 1].append(fk[-1][0:16].astype(F32)[0:8] * 0.0)
                prev = out
            hh_out(_dot(m_ref[pq].astype(BF16), jnp.concatenate(fq, axis=1)), oq, c0, HS)
            kv = _dot_nt(hh_lv(ok, c0, HS), jnp.concatenate(fk, axis=1))
            kv = jnp.where(mkeep, kv, 0.0)
            m_ref[pk] = jnp.where(h % 2 == 0, kv, kv + m_ref[pk])
            w0_ref[...] = w
            l0_ref[...] = lhs
            ao_ref[...] = ao
            al_ref[...] = al
            return c
        lax.fori_loop(0, H, head, 0)
        out = _dot(l0_ref[...], w0_ref[...])
        fin(ao_ref[...] + out[104:128], al_ref[...], H)

    @pl.when(jnp.logical_not(safe))
    def _slow():
        def pair(p, c):
            o40 = pl.multiple_of(p * 40, 8)
            kv = _dot_nt(hh_lv(o40, 0, S), _feat_tile(yt_ref[pl.ds(R_PK + o40, 40), :]))
            m = jnp.where(mkeep, kv, 0.0)
            m_ref[p] = m
            hh_out(_dot(m.astype(BF16), _feat_tile(yt_ref[pl.ds(R_PQ + o40, 40), :])), o40, 0, S)
            return c
        lax.fori_loop(0, H // 2, pair, 0)

        def slow(i, c):
            h = i // (S // 256)
            c0 = pl.multiple_of((i % (S // 256)) * 256, 256)
            ca, cb, off = head_geom(h)
            s = None
            for cw, first in ((ca, True), (cb, False)):
                rows = _iota((128, 256), 0) + (0 if first else 128)
                msk = (rows >= off) & (rows < off + DH)
                if not first:
                    msk = msk & (cb != ca)
                qm = jnp.where(msk, yt_ref[pl.ds(cw, 128), pl.ds(c0, 256)] * QSCALE, 0.0).astype(BF16)
                part = _dot(ks_ref[0:S, pl.ds(cw, 128)], qm)
                s = part if s is None else s + part
            p = jnp.exp2(s - jnp.max(s, axis=0, keepdims=True)).astype(BF16)
            vf = head_rows(R_VA, h)[0:DH]
            c256 = jnp.concatenate([vf, jnp.where(_iota((12, S), 0) == 0, 1.0, 0.0)], axis=0).astype(BF16)
            o = _dot(c256, p)
            o = jnp.concatenate([o[28:32], o[0:DH]], axis=0) * (g_ref[0:1, pl.ds(c0, 256)] / o[DH:DH + 1])
            ota_ref[h + 1, :, pl.ds(c0, 256)] = o
            return c
        lax.fori_loop(0, H * (S // 256), slow, 0)

    c_woa.wait()
    c_wob.wait()

    def ocopy(j):
        r0, r1 = OCH[j]
        return pltpu.make_async_copy(ob_ref.at[pl.ds(r0, r1 - r0), :],
                                     out_hbm.at[pl.ds(r0, r1 - r0), :], osems.at[j])

    for j, (r0, r1) in enumerate(OCH):
        oa = jnp.concatenate([ota_ref[h + 1, 4:4 + DH, r0:r1] for h in range(H)], axis=0).astype(BF16)
        r = lax.dot_general(oa, woa_ref[...], TN, preferred_element_type=F32)
        if j == 0:
            o40 = (H // 2 - 1) * 40
            hh_out(_dot(m_ref[H // 2 - 1].astype(BF16), _feat_tile(yt_ref[R_PQ + o40:R_PQ + o40 + 40, :])),
                   o40, 0, S)
        r = r + lax.dot_general(otb_ref[:, r0:r1].astype(BF16), wob_ref[...], TN,
                                preferred_element_type=F32)
        ob_ref[r0:r1, :] = r.astype(BF16)
        ocopy(j).start()
    for j in range(len(OCH)):
        ocopy(j).wait()


@jax.jit
def pallas_gated_mix__mha_block__linear_kernel_hedgehog__prompt_kernel(
    A_x, A_wqkv, A_wo, B_x, B_wqkv, B_w_phi, B_wo, gate_w
):
    x = A_x.reshape(S, D)
    hbm = pl.BlockSpec(memory_space=pl.ANY)
    out = pl.pallas_call(
        _kernel,
        out_shape=jax.ShapeDtypeStruct((S, D), BF16),
        in_specs=[hbm] * 7,
        out_specs=hbm,
        scratch_shapes=[
            pltpu.VMEM((S, D), BF16),
            pltpu.VMEM((D, D), BF16),
            pltpu.VMEM((D, D), BF16),
            pltpu.VMEM((D, D), BF16),
            pltpu.VMEM((D, 3 * D), BF16),
            pltpu.VMEM((D, D), BF16),
            pltpu.VMEM((D, D), BF16),
            pltpu.VMEM((DH, DH, H), BF16),
            pltpu.VMEM((D,), BF16),
            pltpu.VMEM((S, D), BF16),
            pltpu.SemaphoreType.DMA((11,)),
            pltpu.SemaphoreType.DMA((len(OCH),)),
            pltpu.VMEM((R_END, D), BF16),
            pltpu.VMEM((R_END, S), F32),
            pltpu.VMEM((SP, D), BF16),
            pltpu.VMEM((H + 1, 24, S), F32),
            pltpu.VMEM((D, S), F32),
            pltpu.VMEM((D, 128), F32),
            pltpu.VMEM((8, S), F32),
            pltpu.VMEM((2 * D, 128), F32),
            pltpu.VMEM((8, D), F32),
            pltpu.VMEM((H // 2, 48, 80), F32),
            pltpu.VMEM((128, S), BF16),
            pltpu.VMEM((128, 128), BF16),
            pltpu.VMEM((24, S), F32),
            pltpu.VMEM((8, S), F32),
            pltpu.VMEM((DH, 8, S), F32),
            pltpu.VMEM((len(VROUNDS) * DH, 16, 128), F32),
        ],
        compiler_params=pltpu.CompilerParams(vmem_limit_bytes=120 * 1024 * 1024),
    )(x, A_wqkv, A_wo, B_wqkv, jnp.transpose(B_w_phi, (1, 2, 0)), B_wo, gate_w)
    return out.reshape(1, S, D)
```

```python
import functools
import jax
import jax.numpy as jnp
from jax import lax
from jax.experimental import pallas as pl
from jax.experimental.pallas import tpu as pltpu

S, D, H, DH = 2048, 640, 32, 20
LOG2E = 1.4426950408889634
QSCALE = (DH ** -0.5) * LOG2E
F32, BF16 = jnp.float32, jnp.bfloat16
NT = (((1,), (1,)), ((), ()))
TN = (((0,), (0,)), ((), ()))
R_QA, R_VA, R_PQ, R_PK, R_VB, R_G, R_END = 0, 640, 1280, 1920, 2560, 3200, 3216
KT, NKT = 108, 19
SP = 2080
VP = 2176
VROUNDS = (6, 10, 14, 17)
KM = 92
OCH = ((0, 512), (512, 1024), (1024, 1536), (1536, 1920), (1920, 2048))
HS = S // 2
SCORE_LIMIT = 56.0
V_LO, V_HI = 2.0 ** -36, 2.0 ** 50


def _iota(shape, dim):
    return lax.broadcasted_iota(jnp.int32, shape, dim)


def _dot(a, b):
    return jnp.dot(a, b, preferred_element_type=F32)


def _dot_nt(a, b):
    return lax.dot_general(a, b, NT, preferred_element_type=F32)


def _feat_tile(x, seed=None):
    L = x.shape[1]
    x3 = x.reshape(5, 8, L)

    def allred(v, op):
        v = op(v, pltpu.roll(v, 2, 0))
        return op(v, pltpu.roll(v, 4, 0))
    mx = jnp.max(x3, axis=0)
    mn = jnp.min(x3, axis=0)
    if seed is not None:
        mx = mx + seed
        mn = mn + seed
    mx = allred(mx, jnp.maximum)
    mn = allred(mn, jnp.minimum)
    ep = jnp.exp2(x3 - mx[None])
    en = jnp.exp2(mn[None] - x3)
    rp = 1.0 / allred(jnp.sum(ep, axis=0), jnp.add)
    rn = 1.0 / allred(jnp.sum(en, axis=0), jnp.add)
    return jnp.concatenate([(ep * rp[None]).reshape(40, L), (en * rn[None]).reshape(40, L)],
                           axis=0).astype(BF16)


def _kernel(x_hbm, wa_hbm, woa_hbm, wb_hbm, phi_hbm, wob_hbm, gate_hbm, out_hbm,
            x_ref, wq_ref, wk_ref, wv_ref, wb_ref, woa_ref, wob_ref, phi_ref, gate_ref, ob_ref, sems, osems,
            wt_ref, yt_ref, ks_ref, ota_ref, otb_ref,
            phi2_ref, g_ref, am_ref, km_ref, m_ref, w0_ref, l0_ref, ao_ref, al_ref, qf_ref, kb_ref):
    X0, X1 = 512, 1280

    def xcopy(r0, r1, k):
        return pltpu.make_async_copy(x_hbm.at[pl.ds(r0, r1 - r0), :], x_ref.at[pl.ds(r0, r1 - r0), :], sems.at[k])
    KA = 256
    c_wka = pltpu.make_async_copy(wa_hbm.at[pl.ds(0, KA), pl.ds(D, D)], wk_ref.at[pl.ds(0, KA), :], sems.at[0])
    c_x0a = pltpu.make_async_copy(x_hbm.at[pl.ds(0, X0), pl.ds(0, KA)], x_ref.at[pl.ds(0, X0), pl.ds(0, KA)],
                                  sems.at[1])
    c_wkb = pltpu.make_async_copy(wa_hbm.at[pl.ds(KA, D - KA), pl.ds(D, D)], wk_ref.at[pl.ds(KA, D - KA), :],
                                  sems.at[11])
    c_x0b = pltpu.make_async_copy(x_hbm.at[pl.ds(0, X0), pl.ds(KA, D - KA)],
                                  x_ref.at[pl.ds(0, X0), pl.ds(KA, D - KA)], sems.at[12])
    c_x1 = xcopy(X0, X1, 2)
    c_phi = pltpu.make_async_copy(phi_hbm, phi_ref, sems.at[3])
    c_gate = pltpu.make_async_copy(gate_hbm, gate_ref, sems.at[4])
    c_wq = pltpu.make_async_copy(wa_hbm.at[:, pl.ds(0, D)], wq_ref, sems.at[5])
    c_wv = pltpu.make_async_copy(wa_hbm.at[:, pl.ds(2 * D, D)], wv_ref, sems.at[6])
    c_wb = pltpu.make_async_copy(wb_hbm, wb_ref, sems.at[7])
    c_x2 = xcopy(X1, S, 8)
    c_woa = pltpu.make_async_copy(woa_hbm, woa_ref, sems.at[9])
    c_wob = pltpu.make_async_copy(wob_hbm, wob_ref, sems.at[10])
    for c in (c_wka, c_x0a, c_wkb, c_x0b, c_x1, c_phi, c_gate, c_wq, c_wv, c_x2, c_wb, c_woa, c_wob):
        c.start()

    def proj_k(r0, n, part=None):
        km = None
        for q in range(4):
            a, b = r0 + q * n // 4, r0 + (q + 1) * n // 4
            if part is None:
                k = _dot(x_ref[a:b, :], wk_ref[...])
            else:
                k = part[q] + _dot(x_ref[a:b, KA:D], wk_ref[KA:D, :])
            ks_ref[a:b, :] = k.astype(BF16)
            m = jnp.max(jnp.abs(k).reshape((b - a) // 8, 8, D), axis=0)
            km = m if km is None else jnp.maximum(km, m)
        return km
    ks_ref[S:SP, :] = jnp.zeros((SP - S, D), BF16)
    w0_ref[0:96, :] = jnp.zeros((96, S), BF16)
    ao_ref[...] = jnp.zeros(ao_ref.shape, F32)
    al_ref[...] = jnp.ones(al_ref.shape, F32)
    m_ref[...] = jnp.zeros(m_ref.shape, F32)
    am_ref[...] = jnp.zeros(am_ref.shape, F32)
    c_wka.wait()
    c_x0a.wait()
    for q in range(4):
        a, b = q * X0 // 4, (q + 1) * X0 // 4
        yt_ref[a:b, 0:D] = _dot(x_ref[a:b, 0:KA], wk_ref[0:KA, :])
    c_wkb.wait()
    c_x0b.wait()
    km = proj_k(0, X0, [yt_ref[q * X0 // 4:(q + 1) * X0 // 4, 0:D] for q in range(4)])
    c_x1.wait()
    km = jnp.maximum(km, proj_k(X0, X1 - X0))
    for c in (c_phi, c_gate, c_wq, c_wv, c_x2):
        c.wait()
    km_ref[...] = jnp.maximum(km, proj_k(X1, S - X1))

    for d in range(DH):
        pt = phi_ref[d].astype(F32).T
        phi2_ref[pl.ds(d, H, stride=DH), :] = jnp.concatenate(
            [pt, jnp.zeros((H, 128 - DH), F32)], axis=1)

    wt_ref[R_QA:R_QA + D, :] = wq_ref[...].T
    wt_ref[R_VA:R_VA + D, :] = wv_ref[...].T
    grow = jnp.broadcast_to(gate_ref[...].astype(F32).reshape(1, D), (16, D))
    wt_ref[R_G:R_END, :] = jnp.where(_iota((16, D), 0) == 0, grow, 0.0).astype(BF16)

    c_wb.wait()
    wt_ref[R_VB:R_VB + D, :] = wb_ref[:, 2 * D:3 * D].T

    ri = _iota((128, 128), 0)
    ci = _iota((128, 128), 1)
    sel = ((ri % 40) // 2 == ci).astype(BF16)
    keep = (2 * (ri // 40) + ri % 2 == ci // DH) & (ri < 120)
    for g in range(6):
        n = 120 if g < 5 else 40
        c0 = min(120 * g, D - 128)
        pw = phi2_ref[c0:c0 + 128, :].astype(BF16)
        rep = _dot_nt(sel, pw)
        if g < 5:
            kp = keep
        else:
            kp = (30 + 2 * (ri // 40) + ri % 2 == (c0 + ci) // DH) & (ri < 40)
        lg = jnp.where(kp, rep, 0.0).astype(BF16)[0:(128 if g < 5 else 48)]
        for col0, r0 in ((0, R_PQ), (D, R_PK)):
            fold = _dot_nt(lg, wb_ref[:, col0 + c0:col0 + c0 + 128]) * LOG2E
            yt_ref[r0 - R_PQ + 120 * g:r0 - R_PQ + 120 * g + n, 0:D] = fold[0:n]
    wt_ref[R_PQ:R_VB, :] = yt_ref[0:2 * D, 0:D].astype(BF16)

    def head_rows(r0, hd):
        lo = hd * DH
        w32 = yt_ref[pl.ds(pl.multiple_of(r0 + (lo // 8) * 8, 8), 32), :]
        return jnp.where(hd % 2 == 1, w32[4:28], w32[0:24])

    def head_geom(h):
        lo = h * DH
        a = lo // 128
        return (pl.multiple_of(a * 128, 128), pl.multiple_of(jnp.minimum(a + 1, 4) * 128, 128),
                lo - a * 128)

    sub8 = _iota((8, S), 0)
    lane = _iota((1, 128), 1)

    def q_rows(hd):
        qf = head_rows(R_QA, hd) * QSCALE
        return pltpu.roll(qf[0:8], 4, 0), qf[4:20], qf

    def v_rows(hd):
        return jnp.concatenate([head_rows(R_VA, hd)[0:DH], jnp.zeros((DH, VP - S), F32)], axis=1)

    def k_part(hk, tk, seed=None):
        ca, cb, off = head_geom(hk)
        r0 = (KT * tk) // 16 * 16
        o = KT * tk - r0
        ka = ks_ref[r0:r0 + 128, pl.ds(ca, 128)].astype(F32)[o:o + KT]
        kb = ks_ref[r0:r0 + 128, pl.ds(cb, 128)].astype(F32)[o:o + KT]
        kp = jnp.where(lane >= off, ka, kb)
        if seed is not None:
            kp = kp + seed
        kp = pltpu.roll(kp, (KT + 128 - off) % 128, 1)
        return jnp.where(lane >= KT, kp, 0.0)

    def make_lhs(hk, tk, vf, tv, seed=None):
        kp = k_part(hk, tk, seed)
        if tk in VROUNDS:
            kp = kp[0:KM]
        if vf is not None:
            vp = jnp.where(lane < KT, vf[:, KT * tv:KT * tv + 128], 0.0)
        else:
            vp = jnp.zeros((DH, 128), F32)
        return jnp.concatenate([kp, vp], axis=0).astype(BF16)

    def build_kb(hk, tk, seed=None):
        ca, cb, off = head_geom(hk)
        r0 = (KT * tk + KM) // 16 * 16
        o = KT * tk + KM - r0
        ka = ks_ref[r0:r0 + 32, pl.ds(ca, 128)].astype(F32)[o:o + 16]
        kb = ks_ref[r0:r0 + 32, pl.ds(cb, 128)].astype(F32)[o:o + 16]
        kp = jnp.where(lane >= off, ka, kb)
        if seed is not None:
            kp = kp + seed
        kp = pltpu.roll(kp, (128 - off) % 128, 1)
        kp = jnp.concatenate([pltpu.roll(kp[0:8], 4, 0), pltpu.roll(kp[8:16], 4, 0)], axis=0)
        i = VROUNDS.index(tk)
        for d in range(DH):
            kb_ref[i * DH + d] = jnp.broadcast_to(kp[:, d:d + 1], (16, 128))

    for tv in VROUNDS:
        build_kb(0, tv)
    l0_ref[...] = make_lhs(0, 0, None, 0)

    PC = 256

    def proj_t(j, c):
        off = pl.multiple_of(j * PC, PC)
        y = _dot_nt(wt_ref[...], x_ref[pl.ds(off, PC), :])
        yt_ref[:, pl.ds(off, PC)] = y
        ay = jnp.abs(y[0:2 * D])
        am = jnp.maximum(ay[:, 0:128], ay[:, 128:256])
        am_ref[...] = jnp.maximum(am, am_ref[...])
        return c
    lax.fori_loop(0, S // PC, proj_t, 0)

    kmax = jnp.max(km_ref[...], axis=0, keepdims=True)
    seg = _iota((H, D), 1) // DH == _iota((H, D), 0)
    amat = jnp.where(seg, jnp.broadcast_to(kmax, (H, D)), 0.0).astype(BF16)
    bound = jnp.max(_dot(amat, (am_ref[R_QA:R_QA + D, :] * QSCALE).astype(BF16)))
    vmax = jnp.max(am_ref[R_VA:R_VA + D, :])
    safe = (bound <= SCORE_LIMIT) & (vmax >= V_LO) & (vmax <= V_HI)

    g_ref[...] = jnp.broadcast_to(jax.nn.sigmoid(yt_ref[R_G:R_G + 1, :]), (8, S))

    mr = _iota((48, 80), 0)
    mkeep = jnp.where(mr < 40, mr // DH, mr - 40) == _iota((48, 80), 1) % 2

    def hh_lv(o40, c0, n):
        ones8 = jnp.where(_iota((8, n), 0) < 2, 1.0, 0.0)
        return jnp.concatenate([yt_ref[pl.ds(R_VB + o40, 40), pl.ds(c0, n)], ones8], axis=0).astype(BF16)

    def hh_out(nd, o40, c0, n):
        omg = 1.0 - g_ref[0:1, pl.ds(c0, n)]
        s0 = omg / (nd[40:41, :] + 1e-6)
        s1 = omg / (nd[41:42, :] + 1e-6)
        otb_ref[pl.ds(o40, 40), pl.ds(c0, n)] = nd[0:40, :] * jnp.where(_iota((40, n), 0) < DH, s0, s1)

    def piece(tv, j, seed, kbv):
        a0 = a1 = seed
        for d in range(DH):
            q = qf_ref[d, :, j * 128:(j + 1) * 128]
            a0 = a0 + kbv[d][0:8] * q
            a1 = a1 + kbv[d][8:16] * q
        return jnp.exp2(jnp.concatenate([a0, a1], axis=0))

    todo = [(tv, j) for tv in VROUNDS for j in range(S // 128)]
    plan = {t: [] for t in range(NKT)}
    for n, (tv, j) in enumerate(todo):
        plan[min(int(n * (VROUNDS[-1] - 1) / len(todo)), tv - 2)].append((tv, j))

    def make_w(e, qt, qb):
        return jnp.concatenate([e[0:104], jnp.where(sub8 < 4, e[104:112], qt), qb], axis=0).astype(BF16)

    def fin(ao, al, slot):
        inv = g_ref[0:1, :] / jnp.sum(al, axis=0, keepdims=True)
        ota_ref[slot] = ao * inv

    qt0, qb0, _ = q_rows(0)
    w0_ref[96:128, :] = make_w(jnp.zeros((112, S), F32), qt0, qb0)[96:128]

    @pl.when(safe)
    def _fast():
        def head(h, c):
            hn = jnp.minimum(h + 1, H - 1)
            qt, qb, qf = q_rows(h)
            for d in range(DH):
                qf_ref[d] = jnp.broadcast_to(qf[d:d + 1], (8, S))
            pieces = {}
            ties = {t: [] for t in range(NKT + 2)}
            vf = v_rows(h)
            pk = h // 2
            pq = jnp.maximum(pk - 1, 0)
            c0 = pl.multiple_of((h % 2) * HS, HS)
            ok = pl.multiple_of(pk * 40, 8)
            oq = pl.multiple_of(pq * 40, 8)
            fq, fk = [], []
            w = w0_ref[...]
            lhs = l0_ref[...]
            ao, al = ao_ref[...], al_ref[...]
            prev = None
            for t in range(NKT):
                out = _dot(lhs, w)
                seed = None if prev is None else prev[0:8, 0:128] * 0.0
                useed = None if seed is None else seed[0:1]
                if t + 1 < NKT:
                    lhs = make_lhs(h, t + 1, vf, t, useed)
                else:
                    lhs = make_lhs(hn, 0, vf, t, useed)
                if t in VROUNDS:
                    ao = ao + out[88:112]
                else:
                    ao = ao + out[104:128]
                if t == 0:
                    fin(ao, al, h)
                    ao = jnp.zeros((24, S), F32)
                    al = None
                if t in VROUNDS:
                    ev = jnp.concatenate([pieces.pop((t, j)) for j in range(S // 128)], axis=1)
                    em = jnp.exp2(out[0:96])
                    xr, yr = ev[0:8], ev[8:16]
                    e = jnp.concatenate([em[0:88], jnp.where(sub8 < 4, em[88:96], xr),
                                         jnp.where(sub8 < 4, xr, yr), yr], axis=0)
                    build_kb(hn, t, out[0:1, 128:256] * 0.0)
                else:
                    e = jnp.exp2(out[0:112])
                if ties[t]:
                    top = [e[0:8, 128 * j:128 * (j + 1)] for j in range(S // 128)]
                    for n, v in enumerate(ties[t]):
                        j = (n * (S // 128)) // len(ties[t])
                        top[j] = top[j] + v
                    e = jnp.concatenate([jnp.concatenate(top, axis=1), e[8:112]], axis=0)
                kbs = {tv: [kb_ref[VROUNDS.index(tv) * DH + d] for d in range(DH)] for tv in set(p[0] for p in plan[t])}
                for n, (tv, j) in enumerate(plan[t]):
                    r, cq = (16 * n) % 88, ((n * 16) // max(len(plan[t]), 1)) * 128
                    pieces[(tv, j)] = piece(tv, j, out[r:r + 8, cq:cq + 128] * 0.0, kbs[tv])
                    if t + 1 < tv:
                        ties[t + 1].append(pieces[(tv, j)][0:8] * 0.0)
                last = e[104:112]
                last = jnp.where(sub8 < (4 if t + 1 < NKT else 0), last, 0.0)
                tot = functools.reduce(jnp.add, [e[8 * i:8 * i + 8] for i in range(13)] + [last])
                al = tot if al is None else al + tot
                if t + 1 < NKT:
                    w = make_w(e, qt, qb)
                else:
                    w = make_w(e, *q_rows(hn)[0:2])
                if 2 <= t < 10:
                    u = len(fq)
                    fq.append(_feat_tile(yt_ref[pl.ds(R_PQ + oq, 40), pl.ds(c0 + 128 * u, 128)], seed))
                    ties[t + 1].append(fq[-1][0:16].astype(F32)[0:8] * 0.0)
                elif 10 <= t < 18:
                    u = len(fk)
                    fk.append(_feat_tile(yt_ref[pl.ds(R_PK + ok, 40), pl.ds(c0 + 128 * u, 128)], seed))
                    ties[t + 1].append(fk[-1][0:16].astype(F32)[0:8] * 0.0)
                prev = out
            hh_out(_dot(m_ref[pq].astype(BF16), jnp.concatenate(fq, axis=1)), oq, c0, HS)
            kv = _dot_nt(hh_lv(ok, c0, HS), jnp.concatenate(fk, axis=1))
            kv = jnp.where(mkeep, kv, 0.0)
            m_ref[pk] = jnp.where(h % 2 == 0, kv, kv + m_ref[pk])
            w0_ref[...] = w
            l0_ref[...] = lhs
            ao_ref[...] = ao
            al_ref[...] = al
            return c
        lax.fori_loop(0, H, head, 0)
        out = _dot(l0_ref[...], w0_ref[...])
        fin(ao_ref[...] + out[104:128], al_ref[...], H)

    @pl.when(jnp.logical_not(safe))
    def _slow():
        def pair(p, c):
            o40 = pl.multiple_of(p * 40, 8)
            kv = _dot_nt(hh_lv(o40, 0, S), _feat_tile(yt_ref[pl.ds(R_PK + o40, 40), :]))
            m = jnp.where(mkeep, kv, 0.0)
            m_ref[p] = m
            hh_out(_dot(m.astype(BF16), _feat_tile(yt_ref[pl.ds(R_PQ + o40, 40), :])), o40, 0, S)
            return c
        lax.fori_loop(0, H // 2, pair, 0)

        def slow(i, c):
            h = i // (S // 256)
            c0 = pl.multiple_of((i % (S // 256)) * 256, 256)
            ca, cb, off = head_geom(h)
            s = None
            for cw, first in ((ca, True), (cb, False)):
                rows = _iota((128, 256), 0) + (0 if first else 128)
                msk = (rows >= off) & (rows < off + DH)
                if not first:
                    msk = msk & (cb != ca)
                qm = jnp.where(msk, yt_ref[pl.ds(cw, 128), pl.ds(c0, 256)] * QSCALE, 0.0).astype(BF16)
                part = _dot(ks_ref[0:S, pl.ds(cw, 128)], qm)
                s = part if s is None else s + part
            p = jnp.exp2(s - jnp.max(s, axis=0, keepdims=True)).astype(BF16)
            vf = head_rows(R_VA, h)[0:DH]
            c256 = jnp.concatenate([vf, jnp.where(_iota((12, S), 0) == 0, 1.0, 0.0)], axis=0).astype(BF16)
            o = _dot(c256, p)
            o = jnp.concatenate([o[28:32], o[0:DH]], axis=0) * (g_ref[0:1, pl.ds(c0, 256)] / o[DH:DH + 1])
            ota_ref[h + 1, :, pl.ds(c0, 256)] = o
            return c
        lax.fori_loop(0, H * (S // 256), slow, 0)

    c_woa.wait()
    c_wob.wait()

    def ocopy(j):
        r0, r1 = OCH[j]
        return pltpu.make_async_copy(ob_ref.at[pl.ds(r0, r1 - r0), :],
                                     out_hbm.at[pl.ds(r0, r1 - r0), :], osems.at[j])

    for j, (r0, r1) in enumerate(OCH):
        oa = jnp.concatenate([ota_ref[h + 1, 4:4 + DH, r0:r1] for h in range(H)], axis=0).astype(BF16)
        r = lax.dot_general(oa, woa_ref[...], TN, preferred_element_type=F32)
        if j == 0:
            o40 = (H // 2 - 1) * 40
            hh_out(_dot(m_ref[H // 2 - 1].astype(BF16), _feat_tile(yt_ref[R_PQ + o40:R_PQ + o40 + 40, :])),
                   o40, 0, S)
        r = r + lax.dot_general(otb_ref[:, r0:r1].astype(BF16), wob_ref[...], TN,
                                preferred_element_type=F32)
        ob_ref[r0:r1, :] = r.astype(BF16)
        ocopy(j).start()
    for j in range(len(OCH)):
        ocopy(j).wait()


@jax.jit
def pallas_gated_mix__mha_block__linear_kernel_hedgehog__prompt_kernel(
    A_x, A_wqkv, A_wo, B_x, B_wqkv, B_w_phi, B_wo, gate_w
):
    x = A_x.reshape(S, D)
    hbm = pl.BlockSpec(memory_space=pl.ANY)
    out = pl.pallas_call(
        _kernel,
        out_shape=jax.ShapeDtypeStruct((S, D), BF16),
        in_specs=[hbm] * 7,
        out_specs=hbm,
        scratch_shapes=[
            pltpu.VMEM((S, D), BF16),
            pltpu.VMEM((D, D), BF16),
            pltpu.VMEM((D, D), BF16),
            pltpu.VMEM((D, D), BF16),
            pltpu.VMEM((D, 3 * D), BF16),
            pltpu.VMEM((D, D), BF16),
            pltpu.VMEM((D, D), BF16),
            pltpu.VMEM((DH, DH, H), BF16),
            pltpu.VMEM((D,), BF16),
            pltpu.VMEM((S, D), BF16),
            pltpu.SemaphoreType.DMA((13,)),
            pltpu.SemaphoreType.DMA((len(OCH),)),
            pltpu.VMEM((R_END, D), BF16),
            pltpu.VMEM((R_END, S), F32),
            pltpu.VMEM((SP, D), BF16),
            pltpu.VMEM((H + 1, 24, S), F32),
            pltpu.VMEM((D, S), F32),
            pltpu.VMEM((D, 128), F32),
            pltpu.VMEM((8, S), F32),
            pltpu.VMEM((2 * D, 128), F32),
            pltpu.VMEM((8, D), F32),
            pltpu.VMEM((H // 2, 48, 80), F32),
            pltpu.VMEM((128, S), BF16),
            pltpu.VMEM((128, 128), BF16),
            pltpu.VMEM((24, S), F32),
            pltpu.VMEM((8, S), F32),
            pltpu.VMEM((DH, 8, S), F32),
            pltpu.VMEM((len(VROUNDS) * DH, 16, 128), F32),
        ],
        compiler_params=pltpu.CompilerParams(vmem_limit_bytes=120 * 1024 * 1024),
    )(x, A_wqkv, A_wo, B_wqkv, jnp.transpose(B_w_phi, (1, 2, 0)), B_wo, gate_w)
    return out.reshape(1, S, D)
```

```python
import functools
import jax
import jax.numpy as jnp
from jax import lax
from jax.experimental import pallas as pl
from jax.experimental.pallas import tpu as pltpu

S, D, H, DH = 2048, 640, 32, 20
LOG2E = 1.4426950408889634
QSCALE = (DH ** -0.5) * LOG2E
F32, BF16 = jnp.float32, jnp.bfloat16
NT = (((1,), (1,)), ((), ()))
TN = (((0,), (0,)), ((), ()))
R_QA, R_VA, R_PQ, R_PK, R_VB, R_G, R_END = 0, 640, 1280, 1920, 2560, 3200, 3216
KT, NKT = 108, 19
SP = 2080
VP = 2176
VROUNDS = (6, 10, 14, 17)
KM = 92
OCH = ((0, 512), (512, 1024), (1024, 1536), (1536, 1920), (1920, 2048))
HS = S // 2
SCORE_LIMIT = 56.0
V_LO, V_HI = 2.0 ** -36, 2.0 ** 50


def _iota(shape, dim):
    return lax.broadcasted_iota(jnp.int32, shape, dim)


def _dot(a, b):
    return jnp.dot(a, b, preferred_element_type=F32)


def _dot_nt(a, b):
    return lax.dot_general(a, b, NT, preferred_element_type=F32)


def _feat_tile(x, seed=None):
    L = x.shape[1]
    x3 = x.reshape(5, 8, L)

    def allred(v, op):
        v = op(v, pltpu.roll(v, 2, 0))
        return op(v, pltpu.roll(v, 4, 0))
    mx = jnp.max(x3, axis=0)
    mn = jnp.min(x3, axis=0)
    if seed is not None:
        mx = mx + seed
        mn = mn + seed
    mx = allred(mx, jnp.maximum)
    mn = allred(mn, jnp.minimum)
    ep = jnp.exp2(x3 - mx[None])
    en = jnp.exp2(mn[None] - x3)
    rp = 1.0 / allred(jnp.sum(ep, axis=0), jnp.add)
    rn = 1.0 / allred(jnp.sum(en, axis=0), jnp.add)
    return jnp.concatenate([(ep * rp[None]).reshape(40, L), (en * rn[None]).reshape(40, L)],
                           axis=0).astype(BF16)


def _kernel(x_hbm, wa_hbm, woa_hbm, wb_hbm, phi_hbm, wob_hbm, gate_hbm, out_hbm,
            x_ref, wq_ref, wk_ref, wv_ref, wb_ref, woa_ref, wob_ref, phi_ref, gate_ref, ob_ref, sems, osems,
            wt_ref, yt_ref, ks_ref, ota_ref, otb_ref,
            phi2_ref, g_ref, am_ref, km_ref, m_ref, w0_ref, l0_ref, ao_ref, al_ref, qf_ref, kb_ref):
    X0, X1 = 512, 1280

    def xcopy(r0, r1, k):
        return pltpu.make_async_copy(x_hbm.at[pl.ds(r0, r1 - r0), :], x_ref.at[pl.ds(r0, r1 - r0), :], sems.at[k])
    KA = 256
    c_wka = pltpu.make_async_copy(wa_hbm.at[pl.ds(0, KA), pl.ds(D, D)], wk_ref.at[pl.ds(0, KA), :], sems.at[0])
    c_x0a = pltpu.make_async_copy(x_hbm.at[pl.ds(0, X0), pl.ds(0, KA)], x_ref.at[pl.ds(0, X0), pl.ds(0, KA)],
                                  sems.at[1])
    c_wkb = pltpu.make_async_copy(wa_hbm.at[pl.ds(KA, D - KA), pl.ds(D, D)], wk_ref.at[pl.ds(KA, D - KA), :],
                                  sems.at[11])
    c_x0b = pltpu.make_async_copy(x_hbm.at[pl.ds(0, X0), pl.ds(KA, D - KA)],
                                  x_ref.at[pl.ds(0, X0), pl.ds(KA, D - KA)], sems.at[12])
    c_x1 = xcopy(X0, X1, 2)
    c_phi = pltpu.make_async_copy(phi_hbm, phi_ref, sems.at[3])
    c_gate = pltpu.make_async_copy(gate_hbm, gate_ref, sems.at[4])
    c_wq = pltpu.make_async_copy(wa_hbm.at[:, pl.ds(0, D)], wq_ref, sems.at[5])
    c_wv = pltpu.make_async_copy(wa_hbm.at[:, pl.ds(2 * D, D)], wv_ref, sems.at[6])
    c_wb = pltpu.make_async_copy(wb_hbm, wb_ref, sems.at[7])
    c_x2 = xcopy(X1, S, 8)
    c_woa = pltpu.make_async_copy(woa_hbm, woa_ref, sems.at[9])
    c_wob = pltpu.make_async_copy(wob_hbm, wob_ref, sems.at[10])
    for c in (c_wka, c_x0a, c_wkb, c_x0b, c_x1, c_phi, c_gate, c_wq, c_wv, c_x2, c_wb, c_woa, c_wob):
        c.start()

    def proj_k(r0, n, part=None):
        km = None
        for q in range(4):
            a, b = r0 + q * n // 4, r0 + (q + 1) * n // 4
            if part is None:
                k = _dot(x_ref[a:b, :], wk_ref[...])
            else:
                k = part[q] + _dot(x_ref[a:b, KA:D], wk_ref[KA:D, :])
            ks_ref[a:b, :] = k.astype(BF16)
            m = jnp.max(jnp.abs(k).reshape((b - a) // 8, 8, D), axis=0)
            km = m if km is None else jnp.maximum(km, m)
        return km
    ks_ref[S:SP, :] = jnp.zeros((SP - S, D), BF16)
    w0_ref[0:96, :] = jnp.zeros((96, S), BF16)
    ao_ref[...] = jnp.zeros(ao_ref.shape, F32)
    al_ref[...] = jnp.ones(al_ref.shape, F32)
    m_ref[...] = jnp.zeros(m_ref.shape, F32)
    am_ref[...] = jnp.zeros(am_ref.shape, F32)
    c_wka.wait()
    c_x0a.wait()
    for q in range(4):
        a, b = q * X0 // 4, (q + 1) * X0 // 4
        yt_ref[a:b, 0:D] = _dot(x_ref[a:b, 0:KA], wk_ref[0:KA, :])
    c_wkb.wait()
    c_x0b.wait()
    km = proj_k(0, X0, [yt_ref[q * X0 // 4:(q + 1) * X0 // 4, 0:D] for q in range(4)])
    c_x1.wait()
    km = jnp.maximum(km, proj_k(X0, X1 - X0))
    for c in (c_phi, c_gate, c_wq, c_wv, c_x2):
        c.wait()
    km_ref[...] = jnp.maximum(km, proj_k(X1, S - X1))

    for d in range(DH):
        pt = phi_ref[d].astype(F32).T
        phi2_ref[pl.ds(d, H, stride=DH), :] = jnp.concatenate(
            [pt, jnp.zeros((H, 128 - DH), F32)], axis=1)

    wt_ref[R_QA:R_QA + D, :] = wq_ref[...].T
    wt_ref[R_VA:R_VA + D, :] = wv_ref[...].T
    grow = jnp.broadcast_to(gate_ref[...].astype(F32).reshape(1, D), (16, D))
    wt_ref[R_G:R_END, :] = jnp.where(_iota((16, D), 0) == 0, grow, 0.0).astype(BF16)

    c_wb.wait()
    wt_ref[R_VB:R_VB + D, :] = wb_ref[:, 2 * D:3 * D].T

    ri = _iota((128, 128), 0)
    ci = _iota((128, 128), 1)
    sel = ((ri % 40) // 2 == ci).astype(BF16)
    keep = (2 * (ri // 40) + ri % 2 == ci // DH) & (ri < 120)
    folds = {R_PQ: [], R_PK: []}
    for g in range(6):
        n = 120 if g < 5 else 40
        c0 = min(120 * g, D - 128)
        pw = phi2_ref[c0:c0 + 128, :].astype(BF16)
        rep = _dot_nt(sel, pw)
        if g < 5:
            kp = keep
        else:
            kp = (30 + 2 * (ri // 40) + ri % 2 == (c0 + ci) // DH) & (ri < 40)
        lg = jnp.where(kp, rep, 0.0).astype(BF16)[0:(128 if g < 5 else 48)]
        for col0, r0 in ((0, R_PQ), (D, R_PK)):
            fold = _dot_nt(lg, wb_ref[:, col0 + c0:col0 + c0 + 128]) * LOG2E
            folds[r0].append(fold[0:n])
            if g % 2 == 1:
                blk = jnp.concatenate(folds[r0][-2:], axis=0)
                wt_ref[r0 + 120 * (g - 1):r0 + 120 * (g - 1) + blk.shape[0], :] = blk.astype(BF16)

    def head_rows(r0, hd):
        lo = hd * DH
        w32 = yt_ref[pl.ds(pl.multiple_of(r0 + (lo // 8) * 8, 8), 32), :]
        return jnp.where(hd % 2 == 1, w32[4:28], w32[0:24])

    def head_geom(h):
        lo = h * DH
        a = lo // 128
        return (pl.multiple_of(a * 128, 128), pl.multiple_of(jnp.minimum(a + 1, 4) * 128, 128),
                lo - a * 128)

    sub8 = _iota((8, S), 0)
    lane = _iota((1, 128), 1)

    def q_rows(hd):
        qf = head_rows(R_QA, hd) * QSCALE
        return pltpu.roll(qf[0:8], 4, 0), qf[4:20], qf

    def v_rows(hd):
        return jnp.concatenate([head_rows(R_VA, hd)[0:DH], jnp.zeros((DH, VP - S), F32)], axis=1)

    def k_part(hk, tk, seed=None):
        ca, cb, off = head_geom(hk)
        r0 = (KT * tk) // 16 * 16
        o = KT * tk - r0
        ka = ks_ref[r0:r0 + 128, pl.ds(ca, 128)].astype(F32)[o:o + KT]
        kb = ks_ref[r0:r0 + 128, pl.ds(cb, 128)].astype(F32)[o:o + KT]
        kp = jnp.where(lane >= off, ka, kb)
        if seed is not None:
            kp = kp + seed
        kp = pltpu.roll(kp, (KT + 128 - off) % 128, 1)
        return jnp.where(lane >= KT, kp, 0.0)

    def make_lhs(hk, tk, vf, tv, seed=None):
        kp = k_part(hk, tk, seed)
        if tk in VROUNDS:
            kp = kp[0:KM]
        if vf is not None:
            vp = jnp.where(lane < KT, vf[:, KT * tv:KT * tv + 128], 0.0)
        else:
            vp = jnp.zeros((DH, 128), F32)
        return jnp.concatenate([kp, vp], axis=0).astype(BF16)

    def build_kb(hk, tk, seed=None):
        ca, cb, off = head_geom(hk)
        r0 = (KT * tk + KM) // 16 * 16
        o = KT * tk + KM - r0
        ka = ks_ref[r0:r0 + 32, pl.ds(ca, 128)].astype(F32)[o:o + 16]
        kb = ks_ref[r0:r0 + 32, pl.ds(cb, 128)].astype(F32)[o:o + 16]
        kp = jnp.where(lane >= off, ka, kb)
        if seed is not None:
            kp = kp + seed
        kp = pltpu.roll(kp, (128 - off) % 128, 1)
        kp = jnp.concatenate([pltpu.roll(kp[0:8], 4, 0), pltpu.roll(kp[8:16], 4, 0)], axis=0)
        i = VROUNDS.index(tk)
        for d in range(DH):
            kb_ref[i * DH + d] = jnp.broadcast_to(kp[:, d:d + 1], (16, 128))

    for tv in VROUNDS:
        build_kb(0, tv)
    l0_ref[...] = make_lhs(0, 0, None, 0)

    PC = 256

    def proj_t(j, c):
        off = pl.multiple_of(j * PC, PC)
        y = _dot_nt(wt_ref[...], x_ref[pl.ds(off, PC), :])
        yt_ref[:, pl.ds(off, PC)] = y
        ay = jnp.abs(y[0:2 * D])
        am = jnp.maximum(ay[:, 0:128], ay[:, 128:256])
        am_ref[...] = jnp.maximum(am, am_ref[...])
        return c
    lax.fori_loop(0, S // PC, proj_t, 0)

    kmax = jnp.max(km_ref[...], axis=0, keepdims=True)
    seg = _iota((H, D), 1) // DH == _iota((H, D), 0)
    amat = jnp.where(seg, jnp.broadcast_to(kmax, (H, D)), 0.0).astype(BF16)
    bound = jnp.max(_dot(amat, (am_ref[R_QA:R_QA + D, :] * QSCALE).astype(BF16)))
    vmax = jnp.max(am_ref[R_VA:R_VA + D, :])
    safe = (bound <= SCORE_LIMIT) & (vmax >= V_LO) & (vmax <= V_HI)

    g_ref[...] = jnp.broadcast_to(jax.nn.sigmoid(yt_ref[R_G:R_G + 1, :]), (8, S))

    mr = _iota((48, 80), 0)
    mkeep = jnp.where(mr < 40, mr // DH, mr - 40) == _iota((48, 80), 1) % 2

    def hh_lv(o40, c0, n):
        ones8 = jnp.where(_iota((8, n), 0) < 2, 1.0, 0.0)
        return jnp.concatenate([yt_ref[pl.ds(R_VB + o40, 40), pl.ds(c0, n)], ones8], axis=0).astype(BF16)

    def hh_out(nd, o40, c0, n):
        omg = 1.0 - g_ref[0:1, pl.ds(c0, n)]
        s0 = omg / (nd[40:41, :] + 1e-6)
        s1 = omg / (nd[41:42, :] + 1e-6)
        otb_ref[pl.ds(o40, 40), pl.ds(c0, n)] = nd[0:40, :] * jnp.where(_iota((40, n), 0) < DH, s0, s1)

    def piece(tv, j, seed, kbv):
        a0 = a1 = seed
        for d in range(DH):
            q = qf_ref[d, :, j * 128:(j + 1) * 128]
            a0 = a0 + kbv[d][0:8] * q
            a1 = a1 + kbv[d][8:16] * q
        return jnp.exp2(jnp.concatenate([a0, a1], axis=0))

    todo = [(tv, j) for tv in VROUNDS for j in range(S // 128)]
    plan = {t: [] for t in range(NKT)}
    for n, (tv, j) in enumerate(todo):
        plan[min(int(n * (VROUNDS[-1] - 1) / len(todo)), tv - 2)].append((tv, j))

    def make_w(e, qt, qb):
        return jnp.concatenate([e[0:104], jnp.where(sub8 < 4, e[104:112], qt), qb], axis=0).astype(BF16)

    def fin(ao, al, slot):
        inv = g_ref[0:1, :] / jnp.sum(al, axis=0, keepdims=True)
        ota_ref[slot] = ao * inv

    qt0, qb0, _ = q_rows(0)
    w0_ref[96:128, :] = make_w(jnp.zeros((112, S), F32), qt0, qb0)[96:128]

    @pl.when(safe)
    def _fast():
        def head(h, c):
            hn = jnp.minimum(h + 1, H - 1)
            qt, qb, qf = q_rows(h)
            for d in range(DH):
                qf_ref[d] = jnp.broadcast_to(qf[d:d + 1], (8, S))
            pieces = {}
            ties = {t: [] for t in range(NKT + 2)}
            vf = v_rows(h)
            pk = h // 2
            pq = jnp.maximum(pk - 1, 0)
            c0 = pl.multiple_of((h % 2) * HS, HS)
            ok = pl.multiple_of(pk * 40, 8)
            oq = pl.multiple_of(pq * 40, 8)
            fq, fk = [], []
            w = w0_ref[...]
            lhs = l0_ref[...]
            ao, al = ao_ref[...], al_ref[...]
            prev = None
            for t in range(NKT):
                out = _dot(lhs, w)
                seed = None if prev is None else prev[0:8, 0:128] * 0.0
                useed = None if seed is None else seed[0:1]
                if t + 1 < NKT:
                    lhs = make_lhs(h, t + 1, vf, t, useed)
                else:
                    lhs = make_lhs(hn, 0, vf, t, useed)
                if t in VROUNDS:
                    ao = ao + out[88:112]
                else:
                    ao = ao + out[104:128]
                if t == 0:
                    fin(ao, al, h)
                    ao = jnp.zeros((24, S), F32)
                    al = None
                if t in VROUNDS:
                    ev = jnp.concatenate([pieces.pop((t, j)) for j in range(S // 128)], axis=1)
                    em = jnp.exp2(out[0:96])
                    xr, yr = ev[0:8], ev[8:16]
                    e = jnp.concatenate([em[0:88], jnp.where(sub8 < 4, em[88:96], xr),
                                         jnp.where(sub8 < 4, xr, yr), yr], axis=0)
                    build_kb(hn, t, out[0:1, 128:256] * 0.0)
                else:
                    e = jnp.exp2(out[0:112])
                if ties[t]:
                    top = [e[0:8, 128 * j:128 * (j + 1)] for j in range(S // 128)]
                    for n, v in enumerate(ties[t]):
                        j = (n * (S // 128)) // len(ties[t])
                        top[j] = top[j] + v
                    e = jnp.concatenate([jnp.concatenate(top, axis=1), e[8:112]], axis=0)
                kbs = {tv: [kb_ref[VROUNDS.index(tv) * DH + d] for d in range(DH)] for tv in set(p[0] for p in plan[t])}
                for n, (tv, j) in enumerate(plan[t]):
                    r, cq = (16 * n) % 88, ((n * 16) // max(len(plan[t]), 1)) * 128
                    pieces[(tv, j)] = piece(tv, j, out[r:r + 8, cq:cq + 128] * 0.0, kbs[tv])
                    if t + 1 < tv:
                        ties[t + 1].append(pieces[(tv, j)][0:8] * 0.0)
                last = e[104:112]
                last = jnp.where(sub8 < (4 if t + 1 < NKT else 0), last, 0.0)
                tot = functools.reduce(jnp.add, [e[8 * i:8 * i + 8] for i in range(13)] + [last])
                al = tot if al is None else al + tot
                if t + 1 < NKT:
                    w = make_w(e, qt, qb)
                else:
                    w = make_w(e, *q_rows(hn)[0:2])
                if 2 <= t < 10:
                    u = len(fq)
                    fq.append(_feat_tile(yt_ref[pl.ds(R_PQ + oq, 40), pl.ds(c0 + 128 * u, 128)], seed))
                    ties[t + 1].append(fq[-1][0:16].astype(F32)[0:8] * 0.0)
                elif 10 <= t < 18:
                    u = len(fk)
                    fk.append(_feat_tile(yt_ref[pl.ds(R_PK + ok, 40), pl.ds(c0 + 128 * u, 128)], seed))
                    ties[t + 1].append(fk[-1][0:16].astype(F32)[0:8] * 0.0)
                prev = out
            hh_out(_dot(m_ref[pq].astype(BF16), jnp.concatenate(fq, axis=1)), oq, c0, HS)
            kv = _dot_nt(hh_lv(ok, c0, HS), jnp.concatenate(fk, axis=1))
            kv = jnp.where(mkeep, kv, 0.0)
            m_ref[pk] = jnp.where(h % 2 == 0, kv, kv + m_ref[pk])
            w0_ref[...] = w
            l0_ref[...] = lhs
            ao_ref[...] = ao
            al_ref[...] = al
            return c
        lax.fori_loop(0, H, head, 0)
        out = _dot(l0_ref[...], w0_ref[...])
        fin(ao_ref[...] + out[104:128], al_ref[...], H)

    @pl.when(jnp.logical_not(safe))
    def _slow():
        def pair(p, c):
            o40 = pl.multiple_of(p * 40, 8)
            kv = _dot_nt(hh_lv(o40, 0, S), _feat_tile(yt_ref[pl.ds(R_PK + o40, 40), :]))
            m = jnp.where(mkeep, kv, 0.0)
            m_ref[p] = m
            hh_out(_dot(m.astype(BF16), _feat_tile(yt_ref[pl.ds(R_PQ + o40, 40), :])), o40, 0, S)
            return c
        lax.fori_loop(0, H // 2, pair, 0)

        def slow(i, c):
            h = i // (S // 256)
            c0 = pl.multiple_of((i % (S // 256)) * 256, 256)
            ca, cb, off = head_geom(h)
            s = None
            for cw, first in ((ca, True), (cb, False)):
                rows = _iota((128, 256), 0) + (0 if first else 128)
                msk = (rows >= off) & (rows < off + DH)
                if not first:
                    msk = msk & (cb != ca)
                qm = jnp.where(msk, yt_ref[pl.ds(cw, 128), pl.ds(c0, 256)] * QSCALE, 0.0).astype(BF16)
                part = _dot(ks_ref[0:S, pl.ds(cw, 128)], qm)
                s = part if s is None else s + part
            p = jnp.exp2(s - jnp.max(s, axis=0, keepdims=True)).astype(BF16)
            vf = head_rows(R_VA, h)[0:DH]
            c256 = jnp.concatenate([vf, jnp.where(_iota((12, S), 0) == 0, 1.0, 0.0)], axis=0).astype(BF16)
            o = _dot(c256, p)
            o = jnp.concatenate([o[28:32], o[0:DH]], axis=0) * (g_ref[0:1, pl.ds(c0, 256)] / o[DH:DH + 1])
            ota_ref[h + 1, :, pl.ds(c0, 256)] = o
            return c
        lax.fori_loop(0, H * (S // 256), slow, 0)

    c_woa.wait()
    c_wob.wait()

    def ocopy(j):
        r0, r1 = OCH[j]
        return pltpu.make_async_copy(ob_ref.at[pl.ds(r0, r1 - r0), :],
                                     out_hbm.at[pl.ds(r0, r1 - r0), :], osems.at[j])

    for j, (r0, r1) in enumerate(OCH):
        oa = jnp.concatenate([ota_ref[h + 1, 4:4 + DH, r0:r1] for h in range(H)], axis=0).astype(BF16)
        r = lax.dot_general(oa, woa_ref[...], TN, preferred_element_type=F32)
        if j == 0:
            o40 = (H // 2 - 1) * 40
            hh_out(_dot(m_ref[H // 2 - 1].astype(BF16), _feat_tile(yt_ref[R_PQ + o40:R_PQ + o40 + 40, :])),
                   o40, 0, S)
        r = r + lax.dot_general(otb_ref[:, r0:r1].astype(BF16), wob_ref[...], TN,
                                preferred_element_type=F32)
        ob_ref[r0:r1, :] = r.astype(BF16)
        ocopy(j).start()
    for j in range(len(OCH)):
        ocopy(j).wait()


@jax.jit
def pallas_gated_mix__mha_block__linear_kernel_hedgehog__prompt_kernel(
    A_x, A_wqkv, A_wo, B_x, B_wqkv, B_w_phi, B_wo, gate_w
):
    x = A_x.reshape(S, D)
    hbm = pl.BlockSpec(memory_space=pl.ANY)
    out = pl.pallas_call(
        _kernel,
        out_shape=jax.ShapeDtypeStruct((S, D), BF16),
        in_specs=[hbm] * 7,
        out_specs=hbm,
        scratch_shapes=[
            pltpu.VMEM((S, D), BF16),
            pltpu.VMEM((D, D), BF16),
            pltpu.VMEM((D, D), BF16),
            pltpu.VMEM((D, D), BF16),
            pltpu.VMEM((D, 3 * D), BF16),
            pltpu.VMEM((D, D), BF16),
            pltpu.VMEM((D, D), BF16),
            pltpu.VMEM((DH, DH, H), BF16),
            pltpu.VMEM((D,), BF16),
            pltpu.VMEM((S, D), BF16),
            pltpu.SemaphoreType.DMA((13,)),
            pltpu.SemaphoreType.DMA((len(OCH),)),
            pltpu.VMEM((R_END, D), BF16),
            pltpu.VMEM((R_END, S), F32),
            pltpu.VMEM((SP, D), BF16),
            pltpu.VMEM((H + 1, 24, S), F32),
            pltpu.VMEM((D, S), F32),
            pltpu.VMEM((D, 128), F32),
            pltpu.VMEM((8, S), F32),
            pltpu.VMEM((2 * D, 128), F32),
            pltpu.VMEM((8, D), F32),
            pltpu.VMEM((H // 2, 48, 80), F32),
            pltpu.VMEM((128, S), BF16),
            pltpu.VMEM((128, 128), BF16),
            pltpu.VMEM((24, S), F32),
            pltpu.VMEM((8, S), F32),
            pltpu.VMEM((DH, 8, S), F32),
            pltpu.VMEM((len(VROUNDS) * DH, 16, 128), F32),
        ],
        compiler_params=pltpu.CompilerParams(vmem_limit_bytes=120 * 1024 * 1024),
    )(x, A_wqkv, A_wo, B_wqkv, jnp.transpose(B_w_phi, (1, 2, 0)), B_wo, gate_w)
    return out.reshape(1, S, D)
```
